```python
import jax
import jax.numpy as jnp

def _softmax(x, axis=-1):
    return jax.nn.softmax(x, axis=axis)

def _gelu(x):
    return jax.nn.gelu(x, approximate=True)

def _silu(x):
    return jax.nn.silu(x)

def _sigmoid(x):
    return jax.nn.sigmoid(x)

def _layernorm(x, axis=-1, eps=1e-05):
    m = jnp.mean(x, axis=axis, keepdims=True)
    v = jnp.var(x, axis=axis, keepdims=True)
    return (x - m) / jnp.sqrt(v + eps)

def _scatter_add(tgt, idx, src, axis=0):
    return tgt.at[idx].add(src)

def _segment_sum(src, seg, n):
    return jax.ops.segment_sum(src, seg, n)

class _Rng:

    def __init__(self, key):
        self._k = key

    def _next(self):
        self._k, sub = jax.random.split(self._k)
        return sub

    def normal(self, shape):
        return jax.random.normal(self._next(), shape, dtype=jnp.bfloat16)

    def randint(self, lo, hi, shape):
        return jax.random.randint(self._next(), shape, lo, hi, dtype=jnp.int32)

    def uniform(self, shape, lo=0.0, hi=1.0):
        return jax.random.uniform(self._next(), shape, jnp.bfloat16, lo, hi)

    def permutation(self, n):
        return jax.random.permutation(self._next(), n)
kernel_name = 'recurrent_scan__memory_aug_recurrent_mem_tr__mixer_s_mlp__prompt'

def setup_inputs():
    _rng = _Rng(jax.random.key(int.from_bytes(__import__("os").urandom(4), "little")))
    _w = lambda a: (lambda t: t.astype(jnp.bfloat16) if jnp.issubdtype(t.dtype, jnp.floating) else t)(jnp.asarray(a))

    def _A_setup():
        B, S, Dm = (1, 2048, 1024)
        H, Dh = (32, 128)
        M, seg = (8, 32)
        seg = min(seg, S)
        S = S // seg * seg
        return {'x': _w((lambda *s: _rng.normal(s) * 0.05)(B, S, Dm)), 'mem0': _w((lambda *s: _rng.normal(s) * 0.05)(B, M, Dm)), 'Wq': _w((lambda *s: _rng.normal(s) * 0.05)(Dm, H, Dh) * Dm ** (-0.5)), 'Wk': _w((lambda *s: _rng.normal(s) * 0.05)(Dm, H, Dh) * Dm ** (-0.5)), 'Wv': _w((lambda *s: _rng.normal(s) * 0.05)(Dm, H, Dh) * Dm ** (-0.5)), 'Wo': _w((lambda *s: _rng.normal(s) * 0.05)(H, Dh, Dm) * (H * Dh) ** (-0.5)), 'seg_len': seg}
    _A_in = _A_setup()

    def _B_setup():
        B, S, D, F = (1, 2048, 1024, 3584)
        return {'x': _w((lambda *s: _rng.normal(s) * 0.05)(B, S, D)), 'w1': _w((lambda *s: _rng.normal(s) * 0.05)(D, D) * D ** (-0.5)), 'w2': _w((lambda *s: _rng.normal(s) * 0.05)(D, D) * D ** (-0.5)), 'w3': _w((lambda *s: _rng.normal(s) * 0.05)(D, F) * D ** (-0.5)), 'w4': _w((lambda *s: _rng.normal(s) * 0.05)(F, D) * F ** (-0.5))}
    _B_in = _B_setup()
    return {'A_x': _A_in['x'], 'A_mem0': _A_in['mem0'], 'A_Wq': _A_in['Wq'], 'A_Wk': _A_in['Wk'], 'A_Wv': _A_in['Wv'], 'A_Wo': _A_in['Wo'], 'A_seg_len': _A_in['seg_len'], 'B_x': _B_in['x'], 'B_w1': _B_in['w1'], 'B_w2': _B_in['w2'], 'B_w3': _B_in['w3'], 'B_w4': _B_in['w4']}

def reference(A_x, A_mem0, A_Wq, A_Wk, A_Wv, A_Wo, A_seg_len, B_x, B_w1, B_w2, B_w3, B_w4):

    def _A_ref(x, mem0, Wq, Wk, Wv, Wo, seg_len):
        B, S, Dm = x.shape
        H, Dh = (Wq.shape[1], Wq.shape[2])
        M = mem0.shape[1]
        scale = Dh ** (-0.5)
        n_seg = S // seg_len
        L = M + seg_len
        idx = jnp.arange(L)
        mask = (idx[:, None] < M) | (idx[:, None] >= idx[None, :])
        mem = mem0
        outs = []
        for s in range(n_seg):
            xs = x[:, s * seg_len:(s + 1) * seg_len, :].copy()
            h = jnp.concatenate([mem, xs], axis=1)
            q = jnp.einsum('btd,dhe->bhte', h, Wq)
            k = jnp.einsum('btd,dhe->bhte', h, Wk)
            v = jnp.einsum('btd,dhe->bhte', h, Wv)
            scores = jnp.einsum('bhqe,bhke->bhqk', q, k) * scale
            scores = jnp.where(mask[None, None], scores, -1000000000.0)
            p = _softmax(scores, axis=-1)
            o = jnp.einsum('bhqk,bhke->bhqe', p, v)
            o = jnp.einsum('bhte,hed->btd', o, Wo)
            mem = o[:, :M, :].copy()
            outs.append(o[:, M:, :])
        return jnp.concatenate(outs, axis=1)

    def _B_ref(x, w1, w2, w3, w4):
        B, S, D = x.shape
        h = _gelu(_layernorm(x, axis=-1) @ w1)
        c = D // 4
        g0 = jnp.pad(h[:, :, 0 * c:1 * c], ((0, 0), (1, 0), (0, 0)))[:, :S, :]
        g1 = jnp.pad(h[:, :, 1 * c:2 * c], ((0, 0), (0, 1), (0, 0)))[:, 1:, :]
        g2 = jnp.pad(h[:, :, 2 * c:3 * c], ((0, 0), (2, 0), (0, 0)))[:, :S, :]
        g3 = jnp.pad(h[:, :, 3 * c:], ((0, 0), (0, 2), (0, 0)))[:, 2:, :]
        hs = jnp.concatenate([g0, g1, g2, g3], axis=-1) @ w2
        x1 = x + hs
        h2 = _gelu(_layernorm(x1, axis=-1) @ w3) @ w4
        return x1 + h2
    x = A_x
    xn = _layernorm(x, axis=-1)
    s = _A_ref(xn, A_mem0, A_Wq, A_Wk, A_Wv, A_Wo, A_seg_len)
    g = _silu(_B_ref(xn, B_w1, B_w2, B_w3, B_w4))
    return x + s * g
```

```python
import functools
import math

import jax
import jax.numpy as jnp
import jax.experimental.pallas as pl
import jax.experimental.pallas.tpu as pltpu

F32 = jnp.float32
BF16 = jnp.bfloat16
U32 = jnp.uint32

S, D = 2048, 1024
H, E = 32, 128
M = 8
SEG = 32
FF = 3584
L = M + SEG
SS = 2 * SEG
NSS = S // SS
LROWS = SS + 2 * M
XA = 40
TM = 256
T0 = 512
MF = (S - T0) // NSS
EPS = 1e-5
NEG = -1e30
PITCH = 20
HPAD = 8


def _ln(x):
    m = jnp.mean(x, axis=-1, keepdims=True)
    xc = x - m
    v = jnp.mean(xc * xc, axis=-1, keepdims=True)
    return xc * jax.lax.rsqrt(v + EPS)


def _gelu(x):
    c = math.sqrt(2.0 / math.pi)
    return 0.5 * x * (1.0 + jnp.tanh(c * (x + 0.044715 * (x * x * x))))


def _dot(a, b):
    return jnp.dot(a, b, preferred_element_type=F32)


def _kernel(x_hbm, mem0_ref, wq_hbm, wk_hbm, wv_hbm, wo_hbm, w1_hbm, w2_hbm,
            w3_hbm, w4_hbm, out_hbm,
            xbuf, lhs, x1buf, hbuf, w1, w2, w3t, w4t, wot, raw, wqkv, tmp,
            sem_x, sem_w, sem_raw, sem_out):
    nx = S // TM

    def x_copy(c):
        return pltpu.make_async_copy(x_hbm.at[pl.ds(c * TM, TM)],
                                     xbuf.at[pl.ds(c * TM, TM)], sem_x.at[c])

    def slab_copies(src, dst, sem):
        return [pltpu.make_async_copy(src.at[:, pl.ds(j * 128, 128)], dst.at[j], sem)
                for j in range(dst.shape[0])]

    w1_copy = pltpu.make_async_copy(w1_hbm, w1, sem_w.at[0])
    w2_copy = pltpu.make_async_copy(w2_hbm, w2, sem_w.at[1])
    w3_copies = slab_copies(w3_hbm, w3t, sem_w.at[2])
    w4_copies = slab_copies(w4_hbm, w4t, sem_w.at[3])
    wo_copies = slab_copies(wo_hbm, wot, sem_w.at[4])
    raw_copies = [pltpu.make_async_copy(src, raw.at[i], sem_raw.at[i])
                  for i, src in enumerate((wq_hbm, wk_hbm, wv_hbm))]

    x_copy(0).start()
    w1_copy.start()
    for c in range(1, nx):
        x_copy(c).start()
    w2_copy.start()
    for cp in w3_copies + w4_copies + raw_copies + wo_copies:
        cp.start()

    hbuf[:, 0:HPAD, :] = jnp.zeros((D // 128, HPAD, 128), F32)
    hbuf[:, HPAD + S:HPAD + S + HPAD, :] = jnp.zeros((D // 128, HPAD, 128), F32)
    lhs[0:M, :] = mem0_ref[...]

    w1_copy.wait()

    def p1(c, carry):
        x_copy(c).wait()
        r0 = pl.multiple_of(c * TM, TM)
        xn = _ln(xbuf[pl.ds(r0, TM), :].astype(F32))
        xnb = xn.astype(BF16)
        x1buf[pl.ds(r0, TM), :] = xnb
        for k in range(TM // SS):
            l0 = pl.multiple_of(c * (TM // SS * LROWS) + k * LROWS, 16)
            lhs[pl.ds(l0 + M, XA), :] = xn[k * SS:k * SS + XA].astype(BF16)
            lhs[pl.ds(l0 + 2 * M + XA, SS - XA), :] = xn[k * SS + XA:(k + 1) * SS].astype(BF16)
        z = _ln(xnb.astype(F32)).astype(BF16)
        h = _gelu(_dot(z, w1[...]))
        for n in range(D // 128):
            hbuf[n, pl.ds(r0 + HPAD, TM), :] = h[:, n * 128:(n + 1) * 128]
        return carry

    jax.lax.fori_loop(0, nx, p1, 0)

    w2_copy.wait()

    def p2(c, carry):
        r0 = pl.multiple_of(c * TM, TM)
        g = jnp.concatenate(
            [hbuf[n, pl.ds(r0 + (HPAD + sh), TM), :].astype(BF16)
             for n, sh in enumerate((-1, -1, 1, 1, -2, -2, 2, 2))], axis=1)
        x1 = x1buf[pl.ds(r0, TM), :].astype(F32) + _dot(g, w2[...])
        x1buf[pl.ds(r0, TM), :] = x1.astype(BF16)
        return carry

    jax.lax.fori_loop(0, nx, p2, 0)

    def mlp_up(r0, rows):
        x1 = x1buf[pl.ds(r0, rows), :].astype(F32)
        z = _ln(x1).astype(BF16)
        return jnp.concatenate(
            [_gelu(_dot(z, w3t[j])).astype(BF16) for j in range(FF // 128)], axis=1)

    def mlp_down(r0, rows, u):
        h2 = jnp.concatenate([_dot(u, w4t[n]) for n in range(D // 128)], axis=1)
        y = x1buf[pl.ds(r0, rows), :].astype(F32) + h2
        x1buf[pl.ds(r0, rows), :] = (y * jax.nn.sigmoid(y)).astype(BF16)

    def relayout_block(i, b):
        d0 = pl.multiple_of(b * 16, 16)
        blk = pltpu.bitcast(raw[i, pl.ds(d0, 16)], U32)
        for d in range(16):
            for j in range(2):
                tmp[pl.ds(8 * j * PITCH + d, 8, stride=PITCH), :] = blk[d, 8 * j:8 * j + 8, :]
        r0 = pl.multiple_of(b * 8, 8)
        for hp in range(16):
            a = tmp[pl.ds(hp * PITCH, 8, stride=2), :]
            bb = tmp[pl.ds(hp * PITCH + 1, 8, stride=2), :]
            wqkv[i * H + 2 * hp, pl.ds(r0, 8), :] = (a & U32(0xFFFF)) | (bb << 16)
            wqkv[i * H + 2 * hp + 1, pl.ds(r0, 8), :] = (a >> 16) | (bb & U32(0xFFFF0000))

    for cp in w3_copies + w4_copies:
        cp.wait()

    P3R = 128

    def p3(c, carry):
        r0 = pl.multiple_of(c * P3R, P3R)
        mlp_down(r0, P3R, mlp_up(r0, P3R))
        return carry

    jax.lax.fori_loop(0, T0 // P3R, p3, 0)

    for i in range(3):
        raw_copies[i].wait()

        def rl(b, carry, i=i):
            relayout_block(i, b)
            return carry

        jax.lax.fori_loop(0, D // 16, rl, 0)

    for cp in wo_copies:
        cp.wait()

    ri = jax.lax.broadcasted_iota(jnp.int32, (2 * L, 128), 0)
    ci = jax.lax.broadcasted_iota(jnp.int32, (2 * L, 128), 1)
    second = ri >= L
    rr = jnp.where(second, ri - L, ri)
    cc = jnp.where(second, ci - L, ci)
    valid = (cc >= 0) & (cc < L) & ((rr < M) | (rr >= cc))
    cexp = (E ** -0.5) * math.log2(math.e)
    zpad = jnp.zeros((128 - 2 * L, E), F32)

    def wtile(idx):
        return pltpu.bitcast(wqkv[idx], BF16)

    def attend(q2, k2, v2):
        kp = jnp.concatenate([k2, zpad], axis=0).astype(BF16)
        vp = jnp.concatenate([v2, zpad], axis=0).astype(BF16)
        s = jax.lax.dot_general(q2.astype(BF16), kp, (((1,), (1,)), ((), ())),
                                preferred_element_type=F32)
        s = jnp.where(valid, s, NEG)
        m = jnp.max(s, axis=1, keepdims=True)
        p = jnp.exp2((s - m) * cexp)
        l = jnp.sum(p, axis=1, keepdims=True)
        return _dot(p.astype(BF16), vp) * (1.0 / l)

    GH = 8

    def half_step(h_in, carry_qkv, carry_o):
        step_a = carry_qkv is None
        new_qkv, new_o, og = [], [], []
        acc = None
        for p in range(H // 2):
            qkv = [[], [], []]
            for h in (2 * p, 2 * p + 1):
                for t in range(3):
                    y = _dot(h_in, wtile(t * H + h))
                    if step_a:
                        new_qkv.append(y[L:])
                        qkv[t].append(y[:L])
                    else:
                        c8 = carry_qkv[(h * 3) + t]
                        qkv[t] += [y[:M], c8, y[M:]]
            o2 = attend(*[jnp.concatenate(v, axis=0) for v in qkv])
            for hh in range(2):
                o = o2[hh * L:(hh + 1) * L]
                if step_a:
                    new_o.append(o[L - M:])
                    og.append(o[:L - M].astype(BF16))
                else:
                    og.append(jnp.concatenate([o, carry_o[2 * p + hh]], axis=0).astype(BF16))
            if len(og) == GH:
                g = (2 * p + 2) // GH - 1
                ob = jnp.concatenate(og, axis=1)
                part = jnp.concatenate(
                    [_dot(ob, wot[n, g * GH * E:(g + 1) * GH * E, :]) for n in range(D // 128)],
                    axis=1)
                acc = part if acc is None else acc + part
                og = []
        return acc, new_qkv, new_o

    def out_copy(j):
        r0 = pl.multiple_of(j * SS, SS)
        return pltpu.make_async_copy(xbuf.at[pl.ds(r0, SS)], out_hbm.at[pl.ds(r0, SS)], sem_out)

    def superstep(j, carry):
        l0 = pl.multiple_of(j * LROWS, 16)
        t0 = pl.multiple_of(j * SS, SS)
        f0 = pl.multiple_of(T0 + j * MF, 16)
        acc_a, cq, co = half_step(lhs[pl.ds(l0, M + XA), :], None, None)
        lhs[pl.ds(l0 + M + XA, M), :] = acc_a[:M].astype(BF16)
        u = mlp_up(f0, MF)
        acc_b, _, _ = half_step(lhs[pl.ds(l0 + M + XA, M + SS - XA), :], cq, co)
        lhs[pl.ds(l0 + LROWS, M), :] = acc_b[:M].astype(BF16)
        mlp_down(f0, MF, u)
        s = jnp.concatenate([acc_a[M:], acc_b[L:], acc_b[M:L]], axis=0)
        g = x1buf[pl.ds(t0, SS), :].astype(F32)
        x = xbuf[pl.ds(t0, SS), :].astype(F32)
        xbuf[pl.ds(t0, SS), :] = (x + s * g).astype(BF16)
        out_copy(j).start()
        return carry

    jax.lax.fori_loop(0, NSS, superstep, 0)
    pltpu.make_async_copy(xbuf, out_hbm, sem_out).wait()


@functools.partial(jax.jit, static_argnames=("A_seg_len",))
def pallas_recurrent_scan__memory_aug_recurrent_mem_tr__mixer_s_mlp__prompt_kernel(
    A_x, A_mem0, A_Wq, A_Wk, A_Wv, A_Wo, A_seg_len, B_x, B_w1, B_w2, B_w3, B_w4,
):
    assert A_seg_len == SEG
    assert A_x.shape == (1, S, D) and A_Wq.shape == (D, H, E)
    hbm = pl.BlockSpec(memory_space=pl.ANY)
    out = pl.pallas_call(
        _kernel,
        out_shape=jax.ShapeDtypeStruct((S, D), BF16),
        in_specs=[hbm, pl.BlockSpec(memory_space=pltpu.VMEM)] + [hbm] * 8,
        out_specs=hbm,
        scratch_shapes=[
            pltpu.VMEM((S, D), BF16),
            pltpu.VMEM((NSS * LROWS + 16, D), BF16),
            pltpu.VMEM((S, D), BF16),
            pltpu.VMEM((D // 128, S + 2 * HPAD, 128), F32),
            pltpu.VMEM((D, D), BF16),
            pltpu.VMEM((D, D), BF16),
            pltpu.VMEM((FF // 128, D, 128), BF16),
            pltpu.VMEM((D // 128, FF, 128), BF16),
            pltpu.VMEM((D // 128, H * E, 128), BF16),
            pltpu.VMEM((3, D, H, E), BF16),
            pltpu.VMEM((3 * H, D // 2, E), U32),
            pltpu.VMEM((16 * PITCH, 128), U32),
            pltpu.SemaphoreType.DMA((S // TM,)),
            pltpu.SemaphoreType.DMA((5,)),
            pltpu.SemaphoreType.DMA((3,)),
            pltpu.SemaphoreType.DMA,
        ],
        compiler_params=pltpu.CompilerParams(vmem_limit_bytes=120 * 1024 * 1024),
    )(A_x.reshape(S, D), A_mem0.reshape(M, D), A_Wq, A_Wk, A_Wv,
      A_Wo.reshape(H * E, D), B_w1, B_w2, B_w3, B_w4)
    return out.reshape(1, S, D)
```

```python
import functools
import math

import jax
import jax.numpy as jnp
import jax.experimental.pallas as pl
import jax.experimental.pallas.tpu as pltpu

F32 = jnp.float32
BF16 = jnp.bfloat16
U32 = jnp.uint32

S, D = 2048, 1024
H, E = 32, 128
M = 8
SEG = 32
FF = 3584
L = M + SEG
SS = 2 * SEG
NSS = S // SS
LROWS = SS + 2 * M
XA = 40
TM = 256
T0 = 512
MF = (S - T0) // NSS
EPS = 1e-5
NEG = -1e30
PITCH = 20
NP3 = 4
NTMP = 2
HPAD = 8


def _ln(x):
    m = jnp.mean(x, axis=-1, keepdims=True)
    xc = x - m
    v = jnp.mean(xc * xc, axis=-1, keepdims=True)
    return xc * jax.lax.rsqrt(v + EPS)


def _gelu(x):
    c = math.sqrt(2.0 / math.pi)
    return 0.5 * x * (1.0 + jnp.tanh(c * (x + 0.044715 * (x * x * x))))


def _silu(y):
    h = 0.5 * y
    return h * (1.0 + jnp.tanh(h))


def _dot(a, b):
    return jnp.dot(a, b, preferred_element_type=F32)


def _kernel(x_hbm, mem0_ref, wq_hbm, wk_hbm, wv_hbm, wo_hbm, w1_hbm, w2_hbm,
            w3_hbm, w4_hbm, out_hbm,
            xbuf, obuf, sbuf, lhs, x1buf, hbuf, zbuf, za, zb, w1, w2, w3t, w4t, wot, raw, wqkv, tmp,
            sem_x, sem_w, sem_raw, sem_out):
    nx = S // TM
    RC = 3 * D // NP3

    def x_copy(c):
        return pltpu.make_async_copy(x_hbm.at[pl.ds(c * TM, TM)],
                                     xbuf.at[pl.ds(c * TM, TM)], sem_x.at[c])

    def slab_copies(src, dst, sem):
        return [pltpu.make_async_copy(src.at[:, pl.ds(j * 128, 128)], dst.at[j], sem)
                for j in range(dst.shape[0])]

    w1_copy = pltpu.make_async_copy(w1_hbm, w1, sem_w.at[0])
    w2_copy = pltpu.make_async_copy(w2_hbm, w2, sem_w.at[1])
    w3_copies = slab_copies(w3_hbm, w3t, sem_w.at[2])
    w4_copies = slab_copies(w4_hbm, w4t, sem_w.at[3])
    wo_copies = slab_copies(wo_hbm, wot, sem_w.at[4])
    raw_copies = []
    for i in range(NP3):
        lo, hi = i * RC, (i + 1) * RC
        for w, src in enumerate((wq_hbm, wk_hbm, wv_hbm)):
            a, b = max(lo, w * D), min(hi, (w + 1) * D)
            if a < b:
                raw_copies.append(pltpu.make_async_copy(
                    src.at[pl.ds(a - w * D, b - a)], raw.at[pl.ds(a, b - a)], sem_raw.at[i]))

    x_copy(0).start()
    w1_copy.start()
    for c in range(1, nx):
        x_copy(c).start()
    for cp in [w2_copy] + w3_copies + w4_copies + raw_copies + wo_copies:
        cp.start(priority=1)

    hbuf[:, 0:HPAD, :] = jnp.zeros((D // 128, HPAD, 128), F32)
    hbuf[:, HPAD + S:HPAD + S + HPAD, :] = jnp.zeros((D // 128, HPAD, 128), F32)
    lhs[0:M, :] = mem0_ref[...]

    NPC = 8
    PR = TM // NPC

    def p1_norm_piece(c, k, zout):
        r0 = pl.multiple_of(c * TM + k * PR, PR)
        xn = _ln(xbuf[pl.ds(r0, PR), :].astype(F32))
        xnb = xn.astype(BF16)
        x1buf[pl.ds(r0, PR), :] = xnb
        lbase = pl.multiple_of(c * (TM // SS * LROWS), 16)
        a0 = k * PR
        while a0 < (k + 1) * PR:
            ss, off = divmod(a0, SS)
            if off < XA:
                n = min(XA - off, (k + 1) * PR - a0)
                dst = ss * LROWS + M + off
            else:
                n = min(SS - off, (k + 1) * PR - a0)
                dst = ss * LROWS + 2 * M + off
            lhs[pl.ds(lbase + dst, n), :] = xn[a0 - k * PR:a0 - k * PR + n].astype(BF16)
            a0 += n
        zout[k * PR:(k + 1) * PR, :] = _ln(xnb.astype(F32)).astype(BF16)

    def p1_stage(c_mm, zin, c_norm, zout):
        r0 = pl.multiple_of(c_mm * TM, TM)
        z = zin[...]
        for n in range(D // 128):
            hbuf[n, pl.ds(r0 + HPAD, TM), :] = _gelu(_dot(z, w1[:, n * 128:(n + 1) * 128]))
            if c_norm is not None:
                for k in range(n * NPC // 8, (n + 1) * NPC // 8):
                    p1_norm_piece(c_norm, k, zout)

    x_copy(0).wait()
    for k in range(NPC):
        p1_norm_piece(0, k, za)
    w1_copy.wait()

    def p1(k, carry):
        x_copy(2 * k + 1).wait()
        x_copy(2 * k + 2).wait()
        p1_stage(2 * k, za, 2 * k + 1, zb)
        p1_stage(2 * k + 1, zb, 2 * k + 2, za)
        return carry

    jax.lax.fori_loop(0, nx // 2 - 1, p1, 0)
    x_copy(nx - 1).wait()
    p1_stage(nx - 2, za, nx - 1, zb)
    p1_stage(nx - 1, zb, None, None)

    w2_copy.wait()

    def p2(c, carry):
        r0 = pl.multiple_of(c * TM, TM)
        g = jnp.concatenate(
            [hbuf[n, pl.ds(r0 + (HPAD + sh), TM), :].astype(BF16)
             for n, sh in enumerate((-1, -1, 1, 1, -2, -2, 2, 2))], axis=1)
        x1 = x1buf[pl.ds(r0, TM), :].astype(F32) + _dot(g, w2[...])
        x1buf[pl.ds(r0, TM), :] = x1.astype(BF16)
        return carry

    jax.lax.fori_loop(0, nx, p2, 0)

    def relayout_block(b, slot):
        w = b // (D // 16)
        r0 = pl.multiple_of((b % (D // 16)) * 8, 8)
        d0 = pl.multiple_of(b * 16, 16)
        blk = pltpu.bitcast(raw[pl.ds(d0, 16)], U32)
        for d in range(16):
            for j in range(2):
                tmp[slot, pl.ds(8 * j * PITCH + d, 8, stride=PITCH), :] = blk[d, 8 * j:8 * j + 8, :]
        for hp in range(16):
            a = tmp[slot, pl.ds(hp * PITCH, 8, stride=2), :]
            bb = tmp[slot, pl.ds(hp * PITCH + 1, 8, stride=2), :]
            wqkv[w * H + 2 * hp, pl.ds(r0, 8), :] = (a & U32(0xFFFF)) | (bb << 16)
            wqkv[w * H + 2 * hp + 1, pl.ds(r0, 8), :] = (a >> 16) | (bb & U32(0xFFFF0000))

    P3R = T0 // NP3

    def p3_norm(i):
        r0 = pl.multiple_of(i * P3R, P3R)
        zbuf[i % 2, 0:P3R, :] = _ln(x1buf[pl.ds(r0, P3R), :].astype(F32)).astype(BF16)

    p3_norm(0)
    for cp in w3_copies + w4_copies:
        cp.wait()

    def p3(i, carry):
        c0 = pl.multiple_of(i * RC, 16)
        pltpu.make_async_copy(raw.at[pl.ds(c0, RC)], raw.at[pl.ds(c0, RC)], sem_raw.at[i]).wait()
        r0 = pl.multiple_of(i * P3R, P3R)
        z = zbuf[i % 2, 0:P3R, :]
        p3_norm(i + 1)
        nb = RC // 16
        stages = FF // 128 + D // 128
        done = [0]

        def rl(k):
            upto = nb * k // stages
            for b in range(done[0], upto):
                relayout_block(i * nb + b, b % NTMP)
            done[0] = upto

        us = []
        for j in range(FF // 128):
            us.append(_gelu(_dot(z, w3t[j])).astype(BF16))
            rl(j + 1)
        u = jnp.concatenate(us, axis=1)
        for n in range(D // 128):
            y = x1buf[pl.ds(r0, P3R), n * 128:(n + 1) * 128].astype(F32) + _dot(u, w4t[n])
            x1buf[pl.ds(r0, P3R), n * 128:(n + 1) * 128] = _silu(y).astype(BF16)
            rl(FF // 128 + n + 1)
        return carry

    jax.lax.fori_loop(0, NP3, p3, 0)

    for cp in wo_copies:
        cp.wait()

    ri = jax.lax.broadcasted_iota(jnp.int32, (2 * L, 128), 0)
    ci = jax.lax.broadcasted_iota(jnp.int32, (2 * L, 128), 1)
    second = ri >= L
    rr = jnp.where(second, ri - L, ri)
    cc = jnp.where(second, ci - L, ci)
    valid = (cc >= 0) & (cc < L) & ((rr < M) | (rr >= cc))
    cexp = (E ** -0.5) * math.log2(math.e)
    zpad = jnp.zeros((128 - 2 * L, E), F32)

    def wtile(idx):
        return pltpu.bitcast(wqkv[idx], BF16)

    GH = 8
    NG = H // GH

    def scores(q2, k2):
        kp = jnp.concatenate([k2, zpad], axis=0).astype(BF16)
        return jax.lax.dot_general(q2.astype(BF16), kp, (((1,), (1,)), ((), ())),
                                   preferred_element_type=F32)

    def softmax(s):
        s = jnp.where(valid, s, NEG)
        m = jnp.max(s, axis=1, keepdims=True)
        p = jnp.exp2((s - m) * cexp)
        l = jnp.sum(p, axis=1, keepdims=True)
        r = pl.reciprocal(l, approx=True)
        return p.astype(BF16), r * (2.0 - l * r)

    def half_step(h_in, carry_qkv, carry_o, fillers):
        step_a = carry_qkv is None
        new_qkv, new_o = {}, {}
        rows = {}

        def proj(t, h):
            y = _dot(h_in, wtile(t * H + h))
            if step_a:
                new_qkv[t, h] = y[L:]
                rows[t, h] = [y[:L]]
            else:
                rows[t, h] = [y[:M], carry_qkv[t, h], y[M:]]

        def pair(t, p):
            return jnp.concatenate(rows[t, 2 * p] + rows[t, 2 * p + 1], axis=0)

        def qk(g, half):
            for h in range(g * GH + half * GH // 2, g * GH + (half + 1) * GH // 2):
                proj(0, h)
                proj(1, h)

        def vproj(g):
            for h in range(g * GH, (g + 1) * GH):
                proj(2, h)

        def pairs(g):
            return range(g * GH // 2, (g + 1) * GH // 2)

        def s_stage(g):
            raw_s = [scores(pair(0, p), pair(1, p)) for p in pairs(g)]
            return [softmax(s) for s in raw_s]

        def pv_stage(g, pl_):
            og = []
            o2s = [_dot(pb, jnp.concatenate([pair(2, p), zpad], axis=0).astype(BF16))
                   for p, (pb, _) in zip(pairs(g), pl_)]
            for p, o2, (_, rl) in zip(pairs(g), o2s, pl_):
                o2 = o2 * rl
                for hh in range(2):
                    o = o2[hh * L:(hh + 1) * L]
                    if step_a:
                        new_o[2 * p + hh] = o[L - M:]
                        og.append(o[:L - M].astype(BF16))
                    else:
                        og.append(jnp.concatenate([o, carry_o[2 * p + hh]], axis=0).astype(BF16))
            return jnp.concatenate(og, axis=1)

        def wo_stage(g, ob, acc):
            part = jnp.concatenate(
                [_dot(ob, wot[n, g * GH * E:(g + 1) * GH * E, :]) for n in range(D // 128)],
                axis=1)
            return part if acc is None else acc + part

        acc = None
        qk(0, 0)
        qk(0, 1)
        for g in range(NG):
            last = g == NG - 1
            vproj(g)
            pl_ = s_stage(g)
            fillers[0]() if last else qk(g + 1, 0)
            ob = pv_stage(g, pl_)
            fillers[1]() if last else qk(g + 1, 1)
            acc = wo_stage(g, ob, acc)
        return acc, new_qkv, new_o

    def out_copy(jb):
        return pltpu.make_async_copy(obuf.at[pl.ds(pl.multiple_of(jb * SS, SS), SS)],
                                     out_hbm.at[pl.ds(pl.multiple_of((jb - 1) * SS, SS), SS)],
                                     sem_out)

    def combine(jb):
        t0 = pl.multiple_of(jnp.maximum(jb - 1, 0) * SS, SS)
        g = x1buf[pl.ds(t0, SS), :].astype(F32)
        x = xbuf[pl.ds(t0, SS), :].astype(F32)
        obuf[pl.ds(pl.multiple_of(jb * SS, SS), SS), :] = (x + sbuf[...] * g).astype(BF16)

    sbuf[...] = jnp.zeros((SS, D), F32)

    def superstep(j, carry):
        l0 = pl.multiple_of(j * LROWS, 16)
        f0 = pl.multiple_of(T0 + j * MF, 16)
        combine(j)

        x1 = x1buf[pl.ds(f0, MF), :].astype(F32)
        z = _ln(x1).astype(BF16)
        us = []

        def up(a, b):
            def f():
                for jj in range(a, b):
                    us.append(_gelu(_dot(z, w3t[jj])).astype(BF16))
            return f

        def down(a, b):
            def f():
                u = jnp.concatenate(us, axis=1)
                for n in range(a, b):
                    y = x1[:, n * 128:(n + 1) * 128] + _dot(u, w4t[n])
                    x1buf[pl.ds(f0, MF), n * 128:(n + 1) * 128] = _silu(y).astype(BF16)
            return f

        acc_a, cq, co = half_step(lhs[pl.ds(l0, M + XA), :], None, None, [up(0, 9), up(9, 18)])
        lhs[pl.ds(l0 + M + XA, M), :] = acc_a[:M].astype(BF16)
        sbuf[0:SEG - M, :] = acc_a[M:]
        up(18, 28)()
        acc_b, _, _ = half_step(lhs[pl.ds(l0 + M + XA, M + SS - XA), :], cq, co,
                                [down(0, 3), down(3, 6)])
        lhs[pl.ds(l0 + LROWS, M), :] = acc_b[:M].astype(BF16)
        sbuf[SEG - M:SEG, :] = acc_b[L:]
        sbuf[SEG:SS, :] = acc_b[M:L]
        down(6, 8)()

        @pl.when(j > 0)
        def _():
            out_copy(j).start()

        return carry

    jax.lax.fori_loop(0, NSS, superstep, 0)
    combine(NSS)
    out_copy(NSS).start()
    pltpu.make_async_copy(xbuf, out_hbm, sem_out).wait()


@functools.partial(jax.jit, static_argnames=("A_seg_len",))
def pallas_recurrent_scan__memory_aug_recurrent_mem_tr__mixer_s_mlp__prompt_kernel(
    A_x, A_mem0, A_Wq, A_Wk, A_Wv, A_Wo, A_seg_len, B_x, B_w1, B_w2, B_w3, B_w4,
):
    assert A_seg_len == SEG
    assert A_x.shape == (1, S, D) and A_Wq.shape == (D, H, E)
    hbm = pl.BlockSpec(memory_space=pl.ANY)
    out = pl.pallas_call(
        _kernel,
        out_shape=jax.ShapeDtypeStruct((S, D), BF16),
        in_specs=[hbm, pl.BlockSpec(memory_space=pltpu.VMEM)] + [hbm] * 8,
        out_specs=hbm,
        scratch_shapes=[
            pltpu.VMEM((S, D), BF16),
            pltpu.VMEM((S + SS, D), BF16),
            pltpu.VMEM((SS, D), F32),
            pltpu.VMEM((NSS * LROWS + 16, D), BF16),
            pltpu.VMEM((S, D), BF16),
            pltpu.VMEM((D // 128, S + 2 * HPAD, 128), F32),
            pltpu.VMEM((2, TM, D), BF16),
            pltpu.VMEM((TM, D), BF16),
            pltpu.VMEM((TM, D), BF16),
            pltpu.VMEM((D, D), BF16),
            pltpu.VMEM((D, D), BF16),
            pltpu.VMEM((FF // 128, D, 128), BF16),
            pltpu.VMEM((D // 128, FF, 128), BF16),
            pltpu.VMEM((D // 128, H * E, 128), BF16),
            pltpu.VMEM((3 * D, H, E), BF16),
            pltpu.VMEM((3 * H, D // 2, E), U32),
            pltpu.VMEM((NTMP, 16 * PITCH, 128), U32),
            pltpu.SemaphoreType.DMA((S // TM,)),
            pltpu.SemaphoreType.DMA((5,)),
            pltpu.SemaphoreType.DMA((NP3,)),
            pltpu.SemaphoreType.DMA,
        ],
        compiler_params=pltpu.CompilerParams(vmem_limit_bytes=120 * 1024 * 1024),
    )(A_x.reshape(S, D), A_mem0.reshape(M, D), A_Wq, A_Wk, A_Wv,
      A_Wo.reshape(H * E, D), B_w1, B_w2, B_w3, B_w4)
    return out.reshape(1, S, D)
```

```python
import functools
import math

import jax
import jax.numpy as jnp
import jax.experimental.pallas as pl
import jax.experimental.pallas.tpu as pltpu

F32 = jnp.float32
BF16 = jnp.bfloat16
U32 = jnp.uint32

S, D = 2048, 1024
H, E = 32, 128
M = 8
SEG = 32
FF = 3584
L = M + SEG
SS = 2 * SEG
NSS = S // SS
LROWS = SS + 2 * M
XA = 40
TM = 256
T0 = 512
MF = (S - T0) // NSS
NP3 = 4
P3R = T0 // NP3
RC = 3 * D // NP3
NT = D // 128
NF = FF // 128
EPS = 1e-5
NEG = -1e30
PITCH = 20
NTMP = 2
HPAD = 8
XCUTS = (0, 128, 320, 576, 832, S)

SEM_X = 0
SEM_W1 = SEM_X + len(XCUTS) - 1
SEM_MEM = SEM_W1 + NT
SEM_W2, SEM_W3, SEM_W4, SEM_WO = SEM_MEM + 1, SEM_MEM + 2, SEM_MEM + 3, SEM_MEM + 4
SEM_RAW = SEM_WO + 1
NSEM = SEM_RAW + NP3


def _ln(x):
    m = jnp.mean(x, axis=-1, keepdims=True)
    xc = x - m
    v = jnp.mean(xc * xc, axis=-1, keepdims=True)
    return xc * jax.lax.rsqrt(v + EPS)


def _gelu(x):
    c = math.sqrt(2.0 / math.pi)
    t = jnp.tanh(x * (c + (c * 0.044715) * (x * x)))
    h = 0.5 * x
    return h + h * t


def _silu(y):
    h = 0.5 * y
    return h + h * jnp.tanh(h)


def _dot(a, b):
    return jnp.dot(a, b, preferred_element_type=F32)


def _own_block(i, body):
    return jax.lax.fori_loop(0, jnp.minimum(i + 1, 1), lambda _, c: body(i, c), 0)


def _kernel(x_hbm, mem0_hbm, wq_hbm, wk_hbm, wv_hbm, wo_hbm, w1_hbm, w2_hbm,
            w3_hbm, w4_hbm, out_hbm,
            xbuf, obuf, sbuf, lhs, x1buf, hbuf, zbuf, zc, w1, w2, w3t, w4t, wot, raw, wqkv, tmp,
            sems, sem_out):
    def x_copy(c):
        lo, rows = XCUTS[c], XCUTS[c + 1] - XCUTS[c]
        return pltpu.make_async_copy(x_hbm.at[pl.ds(lo, rows)], xbuf.at[pl.ds(lo, rows)],
                                     sems.at[SEM_X + c])

    def slab_copies(src, dst, sem_of):
        return [pltpu.make_async_copy(src.at[:, pl.ds(j * 128, 128)], dst.at[j], sems.at[sem_of(j)])
                for j in range(dst.shape[0])]

    w1_copies = slab_copies(w1_hbm, w1, lambda j: SEM_W1 + j)
    mem_copy = pltpu.make_async_copy(mem0_hbm, lhs.at[pl.ds(0, M)], sems.at[SEM_MEM])
    w2_copy = pltpu.make_async_copy(w2_hbm, w2, sems.at[SEM_W2])
    w3_copies = slab_copies(w3_hbm, w3t, lambda j: SEM_W3)
    w4_copies = slab_copies(w4_hbm, w4t, lambda j: SEM_W4)
    wo_copies = slab_copies(wo_hbm, wot, lambda j: SEM_WO)
    raw_copies = []
    for i in range(NP3):
        lo, hi = i * RC, (i + 1) * RC
        for w, src in enumerate((wq_hbm, wk_hbm, wv_hbm)):
            a, b = max(lo, w * D), min(hi, (w + 1) * D)
            if a < b:
                raw_copies.append(pltpu.make_async_copy(
                    src.at[pl.ds(a - w * D, b - a)], raw.at[pl.ds(a, b - a)], sems.at[SEM_RAW + i]))

    for cp in ([x_copy(0), x_copy(1)] + w1_copies + [x_copy(c) for c in range(2, len(XCUTS) - 1)]
               + [w2_copy] + w3_copies + w4_copies + raw_copies + [mem_copy] + wo_copies):
        cp.start(priority=1)

    hbuf[:, 0:HPAD, :] = jnp.zeros((NT, HPAD, 128), F32)
    hbuf[:, HPAD + S:HPAD + S + HPAD, :] = jnp.zeros((NT, HPAD, 128), F32)

    PPI = TM // SS

    def ln_piece(p):
        if isinstance(p, int):
            r0, l0 = p * SS, p * LROWS
        else:
            r0, l0 = pl.multiple_of(p * SS, SS), pl.multiple_of(p * LROWS, 16)
        xn = _ln(xbuf[pl.ds(r0, SS), :].astype(F32))
        lhs[pl.ds(l0 + M, XA), :] = xn[:XA].astype(BF16)
        lhs[pl.ds(l0 + 2 * M + XA, SS - XA), :] = xn[XA:].astype(BF16)
        return _ln(xn).astype(BF16)

    x_copy(0).wait()
    z0 = [ln_piece(0), ln_piece(1)]
    x_copy(1).wait()
    z0 = jnp.concatenate(z0 + [ln_piece(2), ln_piece(3)], axis=0)
    for n0 in range(0, NT, 2):
        w1_copies[n0].wait()
        w1_copies[n0 + 1].wait()
        for n in (n0, n0 + 1):
            hbuf[n, HPAD:HPAD + TM, :] = _gelu(_dot(z0, w1[n]))
    zc[...] = ln_piece(PPI)
    x_copy(2).wait()

    def p1(c, carry):
        z = zc[...]
        for q in range(PPI):
            p = c * PPI + q
            pn = jnp.minimum(p + 1, NSS - 1)
            r0 = pl.multiple_of(p * SS, SS)
            znext = ln_piece(pn)
            for n in range(NT):
                hbuf[n, pl.ds(r0 + HPAD, SS), :] = _gelu(_dot(z, w1[n]))
            z = znext
        zc[...] = z

        @pl.when(c == 1)
        def _():
            x_copy(3).wait()

        @pl.when(c == 2)
        def _():
            x_copy(4).wait()

        return carry

    jax.lax.fori_loop(1, S // TM, p1, 0)

    w2_copy.wait()
    P2U = 2

    def p2(cc, carry):
        for k in range(P2U):
            c = cc * P2U + k
            r0 = pl.multiple_of(c * TM, TM)
            g = jnp.concatenate(
                [hbuf[n, pl.ds(r0 + (HPAD + sh), TM), :].astype(BF16)
                 for n, sh in enumerate((-1, -1, 1, 1, -2, -2, 2, 2))], axis=1)
            l0 = pl.multiple_of(c * (PPI * LROWS), 16)
            xn = jnp.concatenate(
                [lhs[pl.ds(l0 + q * LROWS + off, rows), :].astype(F32)
                 for q in range(PPI) for off, rows in ((M, XA), (2 * M + XA, SS - XA))], axis=0)
            x1buf[pl.ds(r0, TM), :] = (xn + _dot(g, w2[...])).astype(BF16)
        return carry

    jax.lax.fori_loop(0, S // TM // P2U, p2, 0)

    def relayout_block(b, slot):
        w = b // (D // 16)
        r0 = pl.multiple_of((b % (D // 16)) * 8, 8)
        d0 = pl.multiple_of(b * 16, 16)
        blk = pltpu.bitcast(raw[pl.ds(d0, 16)], U32)
        for d in range(16):
            for j in range(2):
                tmp[slot, pl.ds(8 * j * PITCH + d, 8, stride=PITCH), :] = blk[d, 8 * j:8 * j + 8, :]
        for hp in range(16):
            a = tmp[slot, pl.ds(hp * PITCH, 8, stride=2), :]
            bb = tmp[slot, pl.ds(hp * PITCH + 1, 8, stride=2), :]
            wqkv[w * H + 2 * hp, pl.ds(r0, 8), :] = (a & U32(0xFFFF)) | (bb << 16)
            wqkv[w * H + 2 * hp + 1, pl.ds(r0, 8), :] = (a >> 16) | (bb & U32(0xFFFF0000))

    def p3_norm(i):
        r0 = pl.multiple_of(i * P3R, P3R)
        z = _ln(x1buf[pl.ds(r0, P3R), :].astype(F32)).astype(BF16)
        zbuf[i % 2] = z

    p3_norm(0)
    for cp in w3_copies + w4_copies:
        cp.wait()

    def p3(i, carry):
        r0 = pl.multiple_of(i * P3R, P3R)
        z = zbuf[i % 2]
        p3_norm(i + 1)
        nb = RC // 16
        stages = NF + NT
        done = 0
        us = []
        for k in range(stages):
            if k < NF:
                us.append(_gelu(_dot(z, w3t[k])).astype(BF16))
            else:
                n = k - NF
                if n == 0:
                    u = jnp.concatenate(us, axis=1)
                y = x1buf[pl.ds(r0, P3R), n * 128:(n + 1) * 128].astype(F32) + _dot(u, w4t[n])
                x1buf[pl.ds(r0, P3R), n * 128:(n + 1) * 128] = _silu(y).astype(BF16)
            upto = nb * (k + 1) // stages
            for b in range(done, upto):
                relayout_block(i * nb + b, b % NTMP)
            done = upto
        return carry

    def p3_outer(i, carry):
        c0 = pl.multiple_of(i * RC, 16)
        pltpu.make_async_copy(raw.at[pl.ds(c0, RC)], raw.at[pl.ds(c0, RC)], sems.at[SEM_RAW + i]).wait()
        return _own_block(i, p3)

    jax.lax.fori_loop(0, NP3, p3_outer, 0)

    mem_copy.wait()
    for cp in wo_copies:
        cp.wait()

    ri = jax.lax.broadcasted_iota(jnp.int32, (2 * L, 128), 0)
    ci = jax.lax.broadcasted_iota(jnp.int32, (2 * L, 128), 1)
    second = ri >= L
    rr = jnp.where(second, ri - L, ri)
    cc = jnp.where(second, ci - L, ci)
    valid = (cc >= 0) & (cc < L) & ((rr < M) | (rr >= cc))
    cexp = (E ** -0.5) * math.log2(math.e)
    zpad = jnp.zeros((128 - 2 * L, E), F32)

    def wtile(idx):
        return pltpu.bitcast(wqkv[idx], BF16)

    GH = 8
    NG = H // GH

    def scores(q2, k2):
        kp = jnp.concatenate([k2, zpad], axis=0).astype(BF16)
        return jax.lax.dot_general(q2.astype(BF16), kp, (((1,), (1,)), ((), ())),
                                   preferred_element_type=F32)

    def softmax(s):
        s = jnp.where(valid, s, NEG)
        m = jnp.max(s, axis=1, keepdims=True)
        p = jnp.exp2((s - m) * cexp)
        l = jnp.sum(p, axis=1, keepdims=True)
        r = pl.reciprocal(l, approx=True)
        return p.astype(BF16), r * (2.0 - l * r)

    def half_step(h_in, carry_qkv, carry_o, fillers):
        step_a = carry_qkv is None
        new_qkv, new_o = {}, {}
        rows = {}

        def proj(t, h):
            y = _dot(h_in, wtile(t * H + h))
            if step_a:
                new_qkv[t, h] = y[L:]
                rows[t, h] = [y[:L]]
            else:
                rows[t, h] = [y[:M], carry_qkv[t, h], y[M:]]

        def pair(t, p):
            return jnp.concatenate(rows[t, 2 * p] + rows[t, 2 * p + 1], axis=0)

        def qk(g, half):
            for h in range(g * GH + half * GH // 2, g * GH + (half + 1) * GH // 2):
                proj(0, h)
                proj(1, h)

        def vproj(g):
            for h in range(g * GH, (g + 1) * GH):
                proj(2, h)

        def pairs(g):
            return range(g * GH // 2, (g + 1) * GH // 2)

        def s_stage(g):
            raw_s = [scores(pair(0, p), pair(1, p)) for p in pairs(g)]
            return [softmax(s) for s in raw_s]

        def pv_stage(g, pl_):
            og = []
            o2s = [_dot(pb, jnp.concatenate([pair(2, p), zpad], axis=0).astype(BF16))
                   for p, (pb, _) in zip(pairs(g), pl_)]
            for p, o2, (_, rl) in zip(pairs(g), o2s, pl_):
                o2 = o2 * rl
                for hh in range(2):
                    o = o2[hh * L:(hh + 1) * L]
                    if step_a:
                        new_o[2 * p + hh] = o[L - M:]
                        og.append(o[:L - M].astype(BF16))
                    else:
                        og.append(jnp.concatenate([o, carry_o[2 * p + hh]], axis=0).astype(BF16))
            return jnp.concatenate(og, axis=1)

        def wo_stage(g, ob, acc):
            part = jnp.concatenate(
                [_dot(ob, wot[n, g * GH * E:(g + 1) * GH * E, :]) for n in range(NT)], axis=1)
            return part if acc is None else acc + part

        acc = None
        qk(0, 0)
        qk(0, 1)
        for g in range(NG):
            last = g == NG - 1
            vproj(g)
            pl_ = s_stage(g)
            fillers[0]() if last else qk(g + 1, 0)
            ob = pv_stage(g, pl_)
            fillers[1]() if last else qk(g + 1, 1)
            acc = wo_stage(g, ob, acc)
        return acc, new_qkv, new_o

    def out_copy(jb):
        return pltpu.make_async_copy(obuf.at[pl.ds(pl.multiple_of(jb * SS, SS), SS)],
                                     out_hbm.at[pl.ds(pl.multiple_of((jb - 1) * SS, SS), SS)],
                                     sem_out)

    def combine(jb):
        t0 = pl.multiple_of(jnp.maximum(jb - 1, 0) * SS, SS)
        g = x1buf[pl.ds(t0, SS), :].astype(F32)
        x = xbuf[pl.ds(t0, SS), :].astype(F32)
        obuf[pl.ds(pl.multiple_of(jb * SS, SS), SS), :] = (x + sbuf[...] * g).astype(BF16)

    sbuf[...] = jnp.zeros((SS, D), F32)
    FS = (9, 18, 3, 6)

    def superstep(j, carry):
        l0 = pl.multiple_of(j * LROWS, 16)
        f0 = pl.multiple_of(T0 + j * MF, 16)
        combine(j)

        x1 = x1buf[pl.ds(f0, MF), :].astype(F32)
        z = _ln(x1).astype(BF16)
        us = []

        def up(a, b):
            def f():
                for jj in range(a, b):
                    us.append(_gelu(_dot(z, w3t[jj])).astype(BF16))
            return f

        def down(a, b):
            def f():
                u = jnp.concatenate(us, axis=1)
                for n in range(a, b):
                    y = x1[:, n * 128:(n + 1) * 128] + _dot(u, w4t[n])
                    x1buf[pl.ds(f0, MF), n * 128:(n + 1) * 128] = _silu(y).astype(BF16)
            return f

        acc_a, cq, co = half_step(lhs[pl.ds(l0, M + XA), :], None, None,
                                  [up(0, FS[0]), up(FS[0], FS[1])])
        lhs[pl.ds(l0 + M + XA, M), :] = acc_a[:M].astype(BF16)
        sbuf[0:SEG - M, :] = acc_a[M:]
        up(FS[1], NF)()
        acc_b, _, _ = half_step(lhs[pl.ds(l0 + M + XA, M + SS - XA), :], cq, co,
                                [down(0, FS[2]), down(FS[2], FS[3])])
        lhs[pl.ds(l0 + LROWS, M), :] = acc_b[:M].astype(BF16)
        sbuf[SEG - M:SEG, :] = acc_b[L:]
        sbuf[SEG:SS, :] = acc_b[M:L]
        down(FS[3], NT)()

        @pl.when(j > 0)
        def _():
            out_copy(j).start(priority=1)

        return carry

    jax.lax.fori_loop(0, NSS, superstep, 0)
    combine(NSS)
    out_copy(NSS).start(priority=1)
    pltpu.make_async_copy(out_hbm, out_hbm, sem_out).wait()


@functools.partial(jax.jit, static_argnames=("A_seg_len",))
def pallas_recurrent_scan__memory_aug_recurrent_mem_tr__mixer_s_mlp__prompt_kernel(
    A_x, A_mem0, A_Wq, A_Wk, A_Wv, A_Wo, A_seg_len, B_x, B_w1, B_w2, B_w3, B_w4,
):
    assert A_seg_len == SEG
    assert A_x.shape == (1, S, D) and A_Wq.shape == (D, H, E)
    hbm = pl.BlockSpec(memory_space=pl.ANY)
    out = pl.pallas_call(
        _kernel,
        out_shape=jax.ShapeDtypeStruct((S, D), BF16),
        in_specs=[hbm] * 10,
        out_specs=hbm,
        scratch_shapes=[
            pltpu.VMEM((S, D), BF16),
            pltpu.VMEM((S + SS, D), BF16),
            pltpu.VMEM((SS, D), F32),
            pltpu.VMEM((NSS * LROWS + 16, D), BF16),
            pltpu.VMEM((S, D), BF16),
            pltpu.VMEM((NT, S + 2 * HPAD, 128), F32),
            pltpu.VMEM((2, P3R, D), BF16),
            pltpu.VMEM((SS, D), BF16),
            pltpu.VMEM((NT, D, 128), BF16),
            pltpu.VMEM((D, D), BF16),
            pltpu.VMEM((NF, D, 128), BF16),
            pltpu.VMEM((NT, FF, 128), BF16),
            pltpu.VMEM((NT, H * E, 128), BF16),
            pltpu.VMEM((3 * D, H, E), BF16),
            pltpu.VMEM((3 * H, D // 2, E), U32),
            pltpu.VMEM((NTMP, 16 * PITCH, 128), U32),
            pltpu.SemaphoreType.DMA((NSEM,)),
            pltpu.SemaphoreType.DMA,
        ],
        compiler_params=pltpu.CompilerParams(vmem_limit_bytes=120 * 1024 * 1024),
    )(A_x.reshape(S, D), A_mem0.reshape(M, D), A_Wq, A_Wk, A_Wv,
      A_Wo.reshape(H * E, D), B_w1, B_w2, B_w3, B_w4)
    return out.reshape(1, S, D)
```

```python
import functools
import math

import jax
import jax.numpy as jnp
import jax.experimental.pallas as pl
import jax.experimental.pallas.tpu as pltpu

F32 = jnp.float32
BF16 = jnp.bfloat16
U32 = jnp.uint32

S, D = 2048, 1024
H, E = 32, 128
M = 8
SEG = 32
FF = 3584
L = M + SEG
SS = 2 * SEG
NSS = S // SS
LROWS = SS + 2 * M
XA = 40
TM = 256
T0 = 512
MF = (S - T0) // NSS
NP3 = 4
P3S = 1
P3R = T0 // NP3 // P3S
RC = 3 * D // NP3
NT = D // 128
NF = FF // 128
EPS = 1e-5
NEG = -1e30
PITCH = 20
NTMP = 2
HPAD = 8
P1N = 7
XCUTS = (0, 128, 320, 320 + 64 * P1N, 320 + 128 * P1N, S)

SEM_X = 0
SEM_W1 = SEM_X + len(XCUTS) - 1
SEM_MEM = SEM_W1 + NT
SEM_W2, SEM_W3, SEM_W4, SEM_WO = SEM_MEM + 1, SEM_MEM + 2, SEM_MEM + 3, SEM_MEM + 4
SEM_RAW = SEM_WO + 1
NSEM = SEM_RAW + NP3


def _ln(x):
    m = jnp.mean(x, axis=-1, keepdims=True)
    xc = x - m
    v = jnp.mean(xc * xc, axis=-1, keepdims=True)
    return xc * jax.lax.rsqrt(v + EPS)


def _gelu(x):
    c = math.sqrt(2.0 / math.pi)
    t = jnp.tanh(x * (c + (c * 0.044715) * (x * x)))
    h = 0.5 * x
    return h + h * t


def _silu(y):
    h = 0.5 * y
    return h + h * jnp.tanh(h)


def _dot(a, b):
    return jnp.dot(a, b, preferred_element_type=F32)


def _own_block(i, body):
    return jax.lax.fori_loop(0, jnp.minimum(i + 1, 1), lambda _, c: body(i, c), 0)


def _kernel(x_hbm, mem0_hbm, wq_hbm, wk_hbm, wv_hbm, wo_hbm, w1_hbm, w2_hbm,
            w3_hbm, w4_hbm, out_hbm,
            xbuf, obuf, sbuf, mbuf, lhs, x1buf, hbuf, zbuf, zc, w1, w2, w3t, w4t, wot, raw, wqkv, tmp,
            sems, sem_out):
    def x_copy(c):
        lo, rows = XCUTS[c], XCUTS[c + 1] - XCUTS[c]
        return pltpu.make_async_copy(x_hbm.at[pl.ds(lo, rows)], xbuf.at[pl.ds(lo, rows)],
                                     sems.at[SEM_X + c])

    def slab_copies(src, dst, sem_of):
        return [pltpu.make_async_copy(src.at[:, pl.ds(j * 128, 128)], dst.at[j], sems.at[sem_of(j)])
                for j in range(dst.shape[0])]

    w1_copies = slab_copies(w1_hbm, w1, lambda j: SEM_W1 + j)
    mem_copy = pltpu.make_async_copy(mem0_hbm, mbuf, sems.at[SEM_MEM])
    w2_copy = pltpu.make_async_copy(w2_hbm, w2, sems.at[SEM_W2])
    w3_copies = slab_copies(w3_hbm, w3t, lambda j: SEM_W3)
    w4_copies = slab_copies(w4_hbm, w4t, lambda j: SEM_W4)
    wo_copies = slab_copies(wo_hbm, wot, lambda j: SEM_WO)
    raw_copies = []
    for i in range(NP3):
        lo, hi = i * RC, (i + 1) * RC
        for w, src in enumerate((wq_hbm, wk_hbm, wv_hbm)):
            a, b = max(lo, w * D), min(hi, (w + 1) * D)
            if a < b:
                raw_copies.append(pltpu.make_async_copy(
                    src.at[pl.ds(a - w * D, b - a)], raw.at[pl.ds(a, b - a)], sems.at[SEM_RAW + i]))

    for cp in ([x_copy(0), x_copy(1)] + w1_copies + [x_copy(c) for c in range(2, len(XCUTS) - 1)]
               + [w2_copy] + w3_copies + w4_copies + raw_copies + [mem_copy] + wo_copies):
        cp.start(priority=1)

    hbuf[:, 0:HPAD, :] = jnp.zeros((NT, HPAD, 128), F32)
    hbuf[:, HPAD + S:HPAD + S + HPAD, :] = jnp.zeros((NT, HPAD, 128), F32)

    PPI = TM // SS

    def ln_piece(p):
        if isinstance(p, int):
            r0, l0 = p * SS, p * LROWS
        else:
            r0, l0 = pl.multiple_of(p * SS, SS), pl.multiple_of(p * LROWS, 16)
        xn = _ln(xbuf[pl.ds(r0, SS), :].astype(F32))
        lhs[pl.ds(l0 + M, XA), :] = xn[:XA].astype(BF16)
        lhs[pl.ds(l0 + 2 * M + XA, SS - XA), :] = xn[XA:].astype(BF16)
        return _ln(xn).astype(BF16)

    x_copy(0).wait()
    z0 = [ln_piece(0), ln_piece(1)]
    x_copy(1).wait()
    z0 = jnp.concatenate(z0 + [ln_piece(2), ln_piece(3)], axis=0)
    for n0 in range(0, NT, 2):
        w1_copies[n0].wait()
        w1_copies[n0 + 1].wait()
        for n in (n0, n0 + 1):
            hbuf[n, HPAD:HPAD + TM, :] = _gelu(_dot(z0, w1[n]))
    zc[...] = ln_piece(PPI)
    x_copy(2).wait()

    def p1(c, carry):
        z = zc[...]
        for q in range(P1N):
            p = PPI + c * P1N + q
            pn = jnp.minimum(p + 1, NSS - 1)
            r0 = pl.multiple_of(p * SS, SS)
            znext = ln_piece(pn)
            for n in range(NT):
                hbuf[n, pl.ds(r0 + HPAD, SS), :] = _gelu(_dot(z, w1[n]))
            z = znext
        zc[...] = z

        @pl.when(c == 0)
        def _():
            x_copy(3).wait()

        @pl.when(c == 1)
        def _():
            x_copy(4).wait()

        return carry

    jax.lax.fori_loop(0, (NSS - PPI) // P1N, p1, 0)

    w2_copy.wait()
    P2U = 2

    def p2(cc, carry):
        for k in range(P2U):
            c = cc * P2U + k
            r0 = pl.multiple_of(c * TM, TM)
            g = jnp.concatenate(
                [hbuf[n, pl.ds(r0 + (HPAD + sh), TM), :].astype(BF16)
                 for n, sh in enumerate((-1, -1, 1, 1, -2, -2, 2, 2))], axis=1)
            l0 = pl.multiple_of(c * (PPI * LROWS), 16)
            xn = jnp.concatenate(
                [lhs[pl.ds(l0 + q * LROWS + off, rows), :].astype(F32)
                 for q in range(PPI) for off, rows in ((M, XA), (2 * M + XA, SS - XA))], axis=0)
            x1buf[pl.ds(r0, TM), :] = (xn + _dot(g, w2[...])).astype(BF16)
        return carry

    jax.lax.fori_loop(0, S // TM // P2U, p2, 0)

    def relayout_block(b, slot):
        w = b // (D // 16)
        r0 = pl.multiple_of((b % (D // 16)) * 8, 8)
        d0 = pl.multiple_of(b * 16, 16)
        blk = pltpu.bitcast(raw[pl.ds(d0, 16)], U32)
        for d in range(16):
            for j in range(2):
                tmp[slot, pl.ds(8 * j * PITCH + d, 8, stride=PITCH), :] = blk[d, 8 * j:8 * j + 8, :]
        for hp in range(16):
            a = tmp[slot, pl.ds(hp * PITCH, 8, stride=2), :]
            bb = tmp[slot, pl.ds(hp * PITCH + 1, 8, stride=2), :]
            wqkv[w * H + 2 * hp, pl.ds(r0, 8), :] = (a & U32(0xFFFF)) | (bb << 16)
            wqkv[w * H + 2 * hp + 1, pl.ds(r0, 8), :] = (a >> 16) | (bb & U32(0xFFFF0000))

    def p3_norm(k):
        r0 = pl.multiple_of(k * P3R, 16)
        return _ln(x1buf[pl.ds(r0, P3R), :].astype(F32)).astype(BF16)

    zbuf[...] = p3_norm(0)
    for cp in w3_copies + w4_copies:
        cp.wait()

    def p3(i, carry):
        nb = RC // 16
        done = 0
        z = zbuf[...]
        for q in range(P3S):
            piece = i * P3S + q
            r0 = pl.multiple_of(piece * P3R, 16)
            znext = p3_norm(piece + 1)
            us = []
            for k in range(NF + NT):
                if k < NF:
                    us.append(_gelu(_dot(z, w3t[k])).astype(BF16))
                else:
                    n = k - NF
                    if n == 0:
                        u = jnp.concatenate(us, axis=1)
                    y = x1buf[pl.ds(r0, P3R), n * 128:(n + 1) * 128].astype(F32) + _dot(u, w4t[n])
                    x1buf[pl.ds(r0, P3R), n * 128:(n + 1) * 128] = _silu(y).astype(BF16)
                if k < NF:
                    upto = 36 * (k + 1) // NF
                else:
                    upto = min(nb, 36 + (nb - 36) * (k - NF + 1) // 6)
                for b in range(done, upto):
                    relayout_block(i * nb + b, b % NTMP)
                done = upto
            z = znext
        zbuf[...] = z
        return carry

    def p3_outer(i, carry):
        c0 = pl.multiple_of(i * RC, 16)
        pltpu.make_async_copy(raw.at[pl.ds(c0, RC)], raw.at[pl.ds(c0, RC)], sems.at[SEM_RAW + i]).wait()
        return _own_block(i, p3)

    jax.lax.fori_loop(0, NP3, p3_outer, 0)

    mem_copy.wait()
    lhs[0:M, :] = mbuf[...]
    for cp in wo_copies:
        cp.wait()

    ri = jax.lax.broadcasted_iota(jnp.int32, (2 * L, 128), 0)
    ci = jax.lax.broadcasted_iota(jnp.int32, (2 * L, 128), 1)
    second = ri >= L
    rr = jnp.where(second, ri - L, ri)
    cc = jnp.where(second, ci - L, ci)
    valid = (cc >= 0) & (cc < L) & ((rr < M) | (rr >= cc))
    cexp = (E ** -0.5) * math.log2(math.e)
    zpad = jnp.zeros((128 - 2 * L, E), F32)

    def wtile(idx):
        return pltpu.bitcast(wqkv[idx], BF16)

    GH = 8
    NG = H // GH

    def scores(q2, k2):
        kp = jnp.concatenate([k2, zpad], axis=0).astype(BF16)
        return jax.lax.dot_general(q2.astype(BF16), kp, (((1,), (1,)), ((), ())),
                                   preferred_element_type=F32)

    def softmax(s):
        s = jnp.where(valid, s, NEG)
        m = jnp.max(s, axis=1, keepdims=True)
        p = jnp.exp2((s - m) * cexp)
        l = jnp.sum(p, axis=1, keepdims=True)
        r = pl.reciprocal(l, approx=True)
        return p.astype(BF16), r * (2.0 - l * r)

    def half_step(h_in, carry_qkv, carry_o, fillers):
        step_a = carry_qkv is None
        new_qkv, new_o = {}, {}
        rows = {}

        def proj(t, h):
            y = _dot(h_in, wtile(t * H + h))
            if step_a:
                new_qkv[t, h] = y[L:]
                rows[t, h] = [y[:L]]
            else:
                rows[t, h] = [y[:M], carry_qkv[t, h], y[M:]]

        def pair(t, p):
            return jnp.concatenate(rows[t, 2 * p] + rows[t, 2 * p + 1], axis=0)

        def qk(g, half):
            for h in range(g * GH + half * GH // 2, g * GH + (half + 1) * GH // 2):
                proj(0, h)
                proj(1, h)

        def vproj(g):
            for h in range(g * GH, (g + 1) * GH):
                proj(2, h)

        def pairs(g):
            return range(g * GH // 2, (g + 1) * GH // 2)

        def s_stage(g):
            raw_s = [scores(pair(0, p), pair(1, p)) for p in pairs(g)]
            return [softmax(s) for s in raw_s]

        def pv_stage(g, pl_):
            og = []
            o2s = [_dot(pb, jnp.concatenate([pair(2, p), zpad], axis=0).astype(BF16))
                   for p, (pb, _) in zip(pairs(g), pl_)]
            for p, o2, (_, rl) in zip(pairs(g), o2s, pl_):
                o2 = o2 * rl
                for hh in range(2):
                    o = o2[hh * L:(hh + 1) * L]
                    if step_a:
                        new_o[2 * p + hh] = o[L - M:]
                        og.append(o[:L - M].astype(BF16))
                    else:
                        og.append(jnp.concatenate([o, carry_o[2 * p + hh]], axis=0).astype(BF16))
            return jnp.concatenate(og, axis=1)

        def wo_stage(g, ob, acc):
            part = jnp.concatenate(
                [_dot(ob, wot[n, g * GH * E:(g + 1) * GH * E, :]) for n in range(NT)], axis=1)
            return part if acc is None else acc + part

        acc = None
        qk(0, 0)
        qk(0, 1)
        for g in range(NG):
            last = g == NG - 1
            vproj(g)
            pl_ = s_stage(g)
            fillers[0]() if last else qk(g + 1, 0)
            ob = pv_stage(g, pl_)
            fillers[1]() if last else qk(g + 1, 1)
            acc = wo_stage(g, ob, acc)
        return acc, new_qkv, new_o

    def out_copy(jb):
        return pltpu.make_async_copy(obuf.at[pl.ds(pl.multiple_of(jb * SS, SS), SS)],
                                     out_hbm.at[pl.ds(pl.multiple_of((jb - 1) * SS, SS), SS)],
                                     sem_out)

    def combine(jb):
        t0 = pl.multiple_of(jnp.maximum(jb - 1, 0) * SS, SS)
        g = x1buf[pl.ds(t0, SS), :].astype(F32)
        x = xbuf[pl.ds(t0, SS), :].astype(F32)
        obuf[pl.ds(pl.multiple_of(jb * SS, SS), SS), :] = (x + sbuf[...] * g).astype(BF16)

    sbuf[...] = jnp.zeros((SS, D), F32)
    FS = (9, 18, 3, 6)

    def superstep(j, carry):
        l0 = pl.multiple_of(j * LROWS, 16)
        f0 = pl.multiple_of(T0 + j * MF, 16)
        combine(j)

        x1 = x1buf[pl.ds(f0, MF), :].astype(F32)
        z = _ln(x1).astype(BF16)
        us = []

        def up(a, b):
            def f():
                for jj in range(a, b):
                    us.append(_gelu(_dot(z, w3t[jj])).astype(BF16))
            return f

        def down(a, b):
            def f():
                u = jnp.concatenate(us, axis=1)
                for n in range(a, b):
                    y = x1[:, n * 128:(n + 1) * 128] + _dot(u, w4t[n])
                    x1buf[pl.ds(f0, MF), n * 128:(n + 1) * 128] = _silu(y).astype(BF16)
            return f

        acc_a, cq, co = half_step(lhs[pl.ds(l0, M + XA), :], None, None,
                                  [up(0, FS[0]), up(FS[0], FS[1])])
        lhs[pl.ds(l0 + M + XA, M), :] = acc_a[:M].astype(BF16)
        sbuf[0:SEG - M, :] = acc_a[M:]
        up(FS[1], NF)()
        acc_b, _, _ = half_step(lhs[pl.ds(l0 + M + XA, M + SS - XA), :], cq, co,
                                [down(0, FS[2]), down(FS[2], FS[3])])
        lhs[pl.ds(l0 + LROWS, M), :] = acc_b[:M].astype(BF16)
        sbuf[SEG - M:SEG, :] = acc_b[L:]
        sbuf[SEG:SS, :] = acc_b[M:L]
        down(FS[3], NT)()

        @pl.when(j > 0)
        def _():
            out_copy(j).start(priority=1)

        return carry

    jax.lax.fori_loop(0, NSS, superstep, 0)
    combine(NSS)
    out_copy(NSS).start(priority=1)
    pltpu.make_async_copy(out_hbm, out_hbm, sem_out).wait()


@functools.partial(jax.jit, static_argnames=("A_seg_len",))
def pallas_recurrent_scan__memory_aug_recurrent_mem_tr__mixer_s_mlp__prompt_kernel(
    A_x, A_mem0, A_Wq, A_Wk, A_Wv, A_Wo, A_seg_len, B_x, B_w1, B_w2, B_w3, B_w4,
):
    assert A_seg_len == SEG
    assert A_x.shape == (1, S, D) and A_Wq.shape == (D, H, E)
    hbm = pl.BlockSpec(memory_space=pl.ANY)
    out = pl.pallas_call(
        _kernel,
        out_shape=jax.ShapeDtypeStruct((S, D), BF16),
        in_specs=[hbm] * 10,
        out_specs=hbm,
        scratch_shapes=[
            pltpu.VMEM((S, D), BF16),
            pltpu.VMEM((S + SS, D), BF16),
            pltpu.VMEM((SS, D), F32),
            pltpu.VMEM((M, D), BF16),
            pltpu.VMEM((NSS * LROWS + 16, D), BF16),
            pltpu.VMEM((S, D), BF16),
            pltpu.VMEM((NT, S + 2 * HPAD, 128), F32),
            pltpu.VMEM((P3R, D), BF16),
            pltpu.VMEM((SS, D), BF16),
            pltpu.VMEM((NT, D, 128), BF16),
            pltpu.VMEM((D, D), BF16),
            pltpu.VMEM((NF, D, 128), BF16),
            pltpu.VMEM((NT, FF, 128), BF16),
            pltpu.VMEM((NT, H * E, 128), BF16),
            pltpu.VMEM((3 * D, H, E), BF16),
            pltpu.VMEM((3 * H, D // 2, E), U32),
            pltpu.VMEM((NTMP, 16 * PITCH, 128), U32),
            pltpu.SemaphoreType.DMA((NSEM,)),
            pltpu.SemaphoreType.DMA,
        ],
        compiler_params=pltpu.CompilerParams(vmem_limit_bytes=120 * 1024 * 1024),
    )(A_x.reshape(S, D), A_mem0.reshape(M, D), A_Wq, A_Wk, A_Wv,
      A_Wo.reshape(H * E, D), B_w1, B_w2, B_w3, B_w4)
    return out.reshape(1, S, D)
```

```python
import functools
import math

import jax
import jax.numpy as jnp
import jax.experimental.pallas as pl
import jax.experimental.pallas.tpu as pltpu

F32 = jnp.float32
BF16 = jnp.bfloat16
U32 = jnp.uint32

S, D = 2048, 1024
H, E = 32, 128
M = 8
SEG = 32
FF = 3584
L = M + SEG
SS = 2 * SEG
NSS = S // SS
LROWS = SS + 2 * M
XA = 40
TM = 256
T0 = 512
MF = (S - T0) // NSS
NP3 = 4
P3S = 1
P3R = T0 // NP3 // P3S
RC = 3 * D // NP3
P3M = 128
NT = D // 128
NF = FF // 128
EPS = 1e-5
NEG = -1e30
PITCH = 20
NTMP = 2
WPAD = 8
HPAD = 8
P1N = 7
XCUTS = (0, 128, 320, 320 + 64 * P1N, 320 + 128 * P1N, S)

SEM_X = 0
SEM_W1 = SEM_X + len(XCUTS) - 1
SEM_MEM = SEM_W1 + NT
SEM_W2, SEM_W3, SEM_W4, SEM_WO = SEM_MEM + 1, SEM_MEM + 2, SEM_MEM + 3, SEM_MEM + 4
SEM_RAW = SEM_WO + 1
NSEM = SEM_RAW + NP3


def _ln(x):
    m = jnp.mean(x, axis=-1, keepdims=True)
    xc = x - m
    v = jnp.mean(xc * xc, axis=-1, keepdims=True)
    return xc * jax.lax.rsqrt(v + EPS)


def _gelu(x):
    c = math.sqrt(2.0 / math.pi)
    t = jnp.tanh(x * (c + (c * 0.044715) * (x * x)))
    h = 0.5 * x
    return h + h * t


def _silu(y):
    h = 0.5 * y
    return h + h * jnp.tanh(h)


def _dot(a, b):
    return jnp.dot(a, b, preferred_element_type=F32)


def _own_block(i, body):
    return jax.lax.fori_loop(0, jnp.minimum(i + 1, 1), lambda _, c: body(i, c), 0)


def _kernel(x_hbm, mem0_hbm, wq_hbm, wk_hbm, wv_hbm, wo_hbm, w1_hbm, w2_hbm,
            w3_hbm, w4_hbm, out_hbm,
            xbuf, obuf, sbuf, mbuf, lhs, x1buf, hbuf, zc, w1, w2, w3t, w4t, wot, raw, wqkv, tmp,
            sems, sem_out):
    def x_copy(c):
        lo, rows = XCUTS[c], XCUTS[c + 1] - XCUTS[c]
        return pltpu.make_async_copy(x_hbm.at[pl.ds(lo, rows)], xbuf.at[pl.ds(lo, rows)],
                                     sems.at[SEM_X + c])

    def slab_copies(src, dst, sem_of):
        return [pltpu.make_async_copy(src.at[:, pl.ds(j * 128, 128)], dst.at[j], sems.at[sem_of(j)])
                for j in range(dst.shape[0])]

    w1_copies = slab_copies(w1_hbm, w1, lambda j: SEM_W1 + j)
    mem_copy = pltpu.make_async_copy(mem0_hbm, mbuf, sems.at[SEM_MEM])
    w2_copy = pltpu.make_async_copy(w2_hbm, w2, sems.at[SEM_W2])
    w3_copies = slab_copies(w3_hbm, w3t, lambda j: SEM_W3)
    w4_copies = slab_copies(w4_hbm, w4t, lambda j: SEM_W4)
    wo_copies = slab_copies(wo_hbm, wot, lambda j: SEM_WO)
    raw_copies = []
    for i in range(NP3):
        lo, hi = i * RC, (i + 1) * RC
        for w, src in enumerate((wq_hbm, wk_hbm, wv_hbm)):
            a, b = max(lo, w * D), min(hi, (w + 1) * D)
            if a < b:
                raw_copies.append(pltpu.make_async_copy(
                    src.at[pl.ds(a - w * D, b - a)], raw.at[pl.ds(a, b - a)], sems.at[SEM_RAW + i]))

    for cp in ([x_copy(0), x_copy(1)] + w1_copies + [x_copy(c) for c in range(2, len(XCUTS) - 1)]
               + [w2_copy] + w3_copies + w4_copies + raw_copies + [mem_copy] + wo_copies):
        cp.start(priority=1)

    hbuf[:, 0:HPAD, :] = jnp.zeros((NT, HPAD, 128), F32)
    hbuf[:, HPAD + S:HPAD + S + HPAD, :] = jnp.zeros((NT, HPAD, 128), F32)

    PPI = TM // SS

    def ln_piece(p):
        if isinstance(p, int):
            r0, l0 = p * SS, p * LROWS
        else:
            r0, l0 = pl.multiple_of(p * SS, SS), pl.multiple_of(p * LROWS, 16)
        xn = _ln(xbuf[pl.ds(r0, SS), :].astype(F32))
        lhs[pl.ds(l0 + M, XA), :] = xn[:XA].astype(BF16)
        lhs[pl.ds(l0 + 2 * M + XA, SS - XA), :] = xn[XA:].astype(BF16)
        return _ln(xn).astype(BF16)

    x_copy(0).wait()
    z0 = [ln_piece(0), ln_piece(1)]
    x_copy(1).wait()
    z0 = jnp.concatenate(z0 + [ln_piece(2), ln_piece(3)], axis=0)
    for n0 in range(0, NT, 2):
        w1_copies[n0].wait()
        w1_copies[n0 + 1].wait()
        for n in (n0, n0 + 1):
            hbuf[n, HPAD:HPAD + TM, :] = _gelu(_dot(z0, w1[n]))
    zc[...] = ln_piece(PPI)
    x_copy(2).wait()

    def p1(c, carry):
        z = zc[...]
        for q in range(P1N):
            p = PPI + c * P1N + q
            pn = jnp.minimum(p + 1, NSS - 1)
            r0 = pl.multiple_of(p * SS, SS)
            znext = ln_piece(pn)
            for n in range(NT):
                hbuf[n, pl.ds(r0 + HPAD, SS), :] = _gelu(_dot(z, w1[n]))
            z = znext
        zc[...] = z

        @pl.when(c == 0)
        def _():
            x_copy(3).wait()

        @pl.when(c == 1)
        def _():
            x_copy(4).wait()

        return carry

    jax.lax.fori_loop(0, (NSS - PPI) // P1N, p1, 0)

    w2_copy.wait()
    P2U = 2

    def mix_rows(r0, pieces):
        rows = pieces * SS
        g = jnp.concatenate(
            [hbuf[n, pl.ds(r0 + (HPAD + sh), rows), :].astype(BF16)
             for n, sh in enumerate((-1, -1, 1, 1, -2, -2, 2, 2))], axis=1)
        l0 = pl.multiple_of((r0 // SS) * LROWS, 16)
        xn = jnp.concatenate(
            [lhs[pl.ds(l0 + q * LROWS + off, n), :].astype(F32)
             for q in range(pieces) for off, n in ((M, XA), (2 * M + XA, SS - XA))], axis=0)
        x1buf[pl.ds(r0, rows), :] = (xn + _dot(g, w2[...])).astype(BF16)

    def p2(cc, carry):
        for k in range(P2U):
            mix_rows(pl.multiple_of((cc * P2U + k) * TM, TM), PPI)
        return carry

    P2ROWS = S - NP3 * P3M
    jax.lax.fori_loop(0, P2ROWS // TM // P2U, p2, 0)

    def relayout_block(b, slot):
        w = b // (D // 16)
        r0 = pl.multiple_of((b % (D // 16)) * 8, 8)
        d0 = pl.multiple_of(b * 16, 16)
        blk = pltpu.bitcast(raw[pl.ds(d0, 16)], U32)
        for d in range(16):
            for j in range(2):
                tmp[slot, pl.ds(8 * j * PITCH + d, 8, stride=PITCH), :] = blk[d, 8 * j:8 * j + 8, :]
        for hp in range(16):
            a = tmp[slot, pl.ds(hp * PITCH, 8, stride=2), :]
            bb = tmp[slot, pl.ds(hp * PITCH + 1, 8, stride=2), :]
            wqkv[w * H + 2 * hp, pl.ds(r0, 8), :] = (a & U32(0xFFFF)) | (bb << 16)
            wqkv[w * H + 2 * hp + 1, pl.ds(r0, 8), :] = (a >> 16) | (bb & U32(0xFFFF0000))

    def p3_norm(k):
        r0 = pl.multiple_of(k * P3R, 16)
        return _ln(x1buf[pl.ds(r0, P3R), :].astype(F32)).astype(BF16)

    for cp in w3_copies + w4_copies:
        cp.wait()

    def p3(i, carry):
        nb = RC // 16
        done = 0
        for q in range(P3S):
            piece = i * P3S + q
            r0 = pl.multiple_of(piece * P3R, 16)
            z = p3_norm(piece)
            mix_rows(pl.multiple_of(P2ROWS + i * P3M, P3M), P3M // SS)
            us = []
            for k in range(NF + NT):
                if k < NF:
                    us.append(_gelu(_dot(z, w3t[k])).astype(BF16))
                else:
                    n = k - NF
                    if n == 0:
                        u = jnp.concatenate(us, axis=1)
                    y = x1buf[pl.ds(r0, P3R), n * 128:(n + 1) * 128].astype(F32) + _dot(u, w4t[n])
                    x1buf[pl.ds(r0, P3R), n * 128:(n + 1) * 128] = _silu(y).astype(BF16)
                if k < NF:
                    upto = 36 * (k + 1) // NF
                else:
                    upto = min(nb, 36 + (nb - 36) * (k - NF + 1) // 6)
                for b in range(done, upto):
                    relayout_block(i * nb + b, b % NTMP)
                done = upto
        return carry

    def p3_outer(i, carry):
        c0 = pl.multiple_of(i * RC, 16)
        pltpu.make_async_copy(raw.at[pl.ds(c0, RC)], raw.at[pl.ds(c0, RC)], sems.at[SEM_RAW + i]).wait()
        return _own_block(i, p3)

    jax.lax.fori_loop(0, NP3, p3_outer, 0)

    mem_copy.wait()
    lhs[0:M, :] = mbuf[...]
    for cp in wo_copies:
        cp.wait()

    ri = jax.lax.broadcasted_iota(jnp.int32, (2 * L, 128), 0)
    ci = jax.lax.broadcasted_iota(jnp.int32, (2 * L, 128), 1)
    second = ri >= L
    rr = jnp.where(second, ri - L, ri)
    cc = jnp.where(second, ci - L, ci)
    valid = (cc >= 0) & (cc < L) & ((rr < M) | (rr >= cc))
    cexp = (E ** -0.5) * math.log2(math.e)
    zpad = jnp.zeros((128 - 2 * L, E), F32)

    def wtile(idx):
        return pltpu.bitcast(wqkv[idx, 0:D // 2, :], BF16)

    GH = 8
    NG = H // GH

    def scores(q2, k2):
        kp = jnp.concatenate([k2, zpad], axis=0).astype(BF16)
        return jax.lax.dot_general(q2.astype(BF16), kp, (((1,), (1,)), ((), ())),
                                   preferred_element_type=F32)

    def softmax(s):
        s = jnp.where(valid, s, NEG)
        m = jnp.max(s, axis=1, keepdims=True)
        p = jnp.exp2((s - m) * cexp)
        l = jnp.sum(p, axis=1, keepdims=True)
        r = pl.reciprocal(l, approx=True)
        return p.astype(BF16), r * (2.0 - l * r)

    def half_step(h_in, carry_qkv, carry_o, fillers):
        step_a = carry_qkv is None
        new_qkv, new_o = {}, {}
        rows = {}

        def proj(t, h):
            y = _dot(h_in, wtile(t * H + h))
            if step_a:
                new_qkv[t, h] = y[L:]
                rows[t, h] = [y[:L]]
            else:
                rows[t, h] = [y[:M], carry_qkv[t, h], y[M:]]

        def pair(t, p):
            return jnp.concatenate(rows[t, 2 * p] + rows[t, 2 * p + 1], axis=0)

        def qk(g, half):
            for h in range(g * GH + half * GH // 2, g * GH + (half + 1) * GH // 2):
                proj(0, h)
                proj(1, h)

        def vproj(g):
            for h in range(g * GH, (g + 1) * GH):
                proj(2, h)

        def pairs(g):
            return range(g * GH // 2, (g + 1) * GH // 2)

        def s_stage(g):
            raw_s = [scores(pair(0, p), pair(1, p)) for p in pairs(g)]
            return [softmax(s) for s in raw_s]

        def pv_stage(g, pl_):
            og = []
            o2s = [_dot(pb, jnp.concatenate([pair(2, p), zpad], axis=0).astype(BF16))
                   for p, (pb, _) in zip(pairs(g), pl_)]
            for p, o2, (_, rl) in zip(pairs(g), o2s, pl_):
                o2 = o2 * rl
                for hh in range(2):
                    o = o2[hh * L:(hh + 1) * L]
                    if step_a:
                        new_o[2 * p + hh] = o[L - M:]
                        og.append(o[:L - M].astype(BF16))
                    else:
                        og.append(jnp.concatenate([o, carry_o[2 * p + hh]], axis=0).astype(BF16))
            return jnp.concatenate(og, axis=1)

        def wo_stage(g, ob, acc):
            part = jnp.concatenate(
                [_dot(ob, wot[n, g * GH * E:(g + 1) * GH * E, :]) for n in range(NT)], axis=1)
            return part if acc is None else acc + part

        acc = None
        qk(0, 0)
        qk(0, 1)
        for g in range(NG):
            last = g == NG - 1
            vproj(g)
            pl_ = s_stage(g)
            fillers[0]() if last else qk(g + 1, 0)
            ob = pv_stage(g, pl_)
            fillers[1]() if last else qk(g + 1, 1)
            acc = wo_stage(g, ob, acc)
        return acc, new_qkv, new_o

    def out_copy(jb):
        return pltpu.make_async_copy(obuf.at[pl.ds(pl.multiple_of(jb * SS, SS), SS)],
                                     out_hbm.at[pl.ds(pl.multiple_of((jb - 1) * SS, SS), SS)],
                                     sem_out)

    def combine(jb):
        t0 = pl.multiple_of(jnp.maximum(jb - 1, 0) * SS, SS)
        g = x1buf[pl.ds(t0, SS), :].astype(F32)
        x = xbuf[pl.ds(t0, SS), :].astype(F32)
        obuf[pl.ds(pl.multiple_of(jb * SS, SS), SS), :] = (x + sbuf[...] * g).astype(BF16)

    sbuf[...] = jnp.zeros((SS, D), F32)
    FS = (9, 18, 3, 6)

    def superstep(j, carry):
        l0 = pl.multiple_of(j * LROWS, 16)
        f0 = pl.multiple_of(T0 + j * MF, 16)
        combine(j)

        x1 = x1buf[pl.ds(f0, MF), :].astype(F32)
        z = _ln(x1).astype(BF16)
        us = []

        def up(a, b):
            def f():
                for jj in range(a, b):
                    us.append(_gelu(_dot(z, w3t[jj])).astype(BF16))
            return f

        def down(a, b):
            def f():
                u = jnp.concatenate(us, axis=1)
                for n in range(a, b):
                    y = x1[:, n * 128:(n + 1) * 128] + _dot(u, w4t[n])
                    x1buf[pl.ds(f0, MF), n * 128:(n + 1) * 128] = _silu(y).astype(BF16)
            return f

        acc_a, cq, co = half_step(lhs[pl.ds(l0, M + XA), :], None, None,
                                  [up(0, FS[0]), up(FS[0], FS[1])])
        lhs[pl.ds(l0 + M + XA, M), :] = acc_a[:M].astype(BF16)
        sbuf[0:SEG - M, :] = acc_a[M:]
        up(FS[1], NF)()
        acc_b, _, _ = half_step(lhs[pl.ds(l0 + M + XA, M + SS - XA), :], cq, co,
                                [down(0, FS[2]), down(FS[2], FS[3])])
        lhs[pl.ds(l0 + LROWS, M), :] = acc_b[:M].astype(BF16)
        sbuf[SEG - M:SEG, :] = acc_b[L:]
        sbuf[SEG:SS, :] = acc_b[M:L]
        down(FS[3], NT)()

        @pl.when(j > 0)
        def _():
            out_copy(j).start(priority=1)

        return carry

    jax.lax.fori_loop(0, NSS, superstep, 0)
    combine(NSS)
    out_copy(NSS).start(priority=1)
    pltpu.make_async_copy(out_hbm, out_hbm, sem_out).wait()


@functools.partial(jax.jit, static_argnames=("A_seg_len",))
def pallas_recurrent_scan__memory_aug_recurrent_mem_tr__mixer_s_mlp__prompt_kernel(
    A_x, A_mem0, A_Wq, A_Wk, A_Wv, A_Wo, A_seg_len, B_x, B_w1, B_w2, B_w3, B_w4,
):
    assert A_seg_len == SEG
    assert A_x.shape == (1, S, D) and A_Wq.shape == (D, H, E)
    hbm = pl.BlockSpec(memory_space=pl.ANY)
    out = pl.pallas_call(
        _kernel,
        out_shape=jax.ShapeDtypeStruct((S, D), BF16),
        in_specs=[hbm] * 10,
        out_specs=hbm,
        scratch_shapes=[
            pltpu.VMEM((S, D), BF16),
            pltpu.VMEM((S + SS, D), BF16),
            pltpu.VMEM((SS, D), F32),
            pltpu.VMEM((M, D), BF16),
            pltpu.VMEM((NSS * LROWS + 16, D), BF16),
            pltpu.VMEM((S, D), BF16),
            pltpu.VMEM((NT, S + 2 * HPAD, 128), F32),
            pltpu.VMEM((SS, D), BF16),
            pltpu.VMEM((NT, D, 128), BF16),
            pltpu.VMEM((D, D), BF16),
            pltpu.VMEM((NF, D, 128), BF16),
            pltpu.VMEM((NT, FF, 128), BF16),
            pltpu.VMEM((NT, H * E, 128), BF16),
            pltpu.VMEM((3 * D, H, E), BF16),
            pltpu.VMEM((3 * H, D // 2 + WPAD, E), U32),
            pltpu.VMEM((NTMP, 16 * PITCH, 128), U32),
            pltpu.SemaphoreType.DMA((NSEM,)),
            pltpu.SemaphoreType.DMA,
        ],
        compiler_params=pltpu.CompilerParams(vmem_limit_bytes=120 * 1024 * 1024),
    )(A_x.reshape(S, D), A_mem0.reshape(M, D), A_Wq, A_Wk, A_Wv,
      A_Wo.reshape(H * E, D), B_w1, B_w2, B_w3, B_w4)
    return out.reshape(1, S, D)
```

```python
import math

import jax
import jax.numpy as jnp
import jax.experimental.pallas as pl
import jax.experimental.pallas.tpu as pltpu

F32 = jnp.float32
BF16 = jnp.bfloat16
U32 = jnp.uint32

S, D = 2048, 1024
H, E = 32, 128
M = 8
SEG = 32
FF = 3584
L = M + SEG
SS = 2 * SEG
NSS = S // SS
LROWS = SS + 2 * M
XA = 40
TM = 256
T0 = 512
MF = (S - T0) // NSS
NP3 = 4
P3R = T0 // NP3
RC = 3 * D // NP3
P3M = 128
NT = D // 128
NF = FF // 128
EPS = 1e-5
NEG = -1e30
PITCH = 20
NTMP = 2
WPAD = 8
HPAD = 8
P1N = 7
XCUTS = (0, 128, 320, 320 + 64 * P1N, 320 + 128 * P1N, S)

SEM_X = 0
SEM_W1 = SEM_X + len(XCUTS) - 1
SEM_MEM = SEM_W1 + NT
SEM_W2, SEM_W3, SEM_W4, SEM_WO = SEM_MEM + 1, SEM_MEM + 2, SEM_MEM + 3, SEM_MEM + 4
SEM_RAW = SEM_WO + 1
NSEM = SEM_RAW + NP3


def _ln(x):
    m = jnp.mean(x, axis=-1, keepdims=True)
    xc = x - m
    v = jnp.mean(xc * xc, axis=-1, keepdims=True)
    return xc * jax.lax.rsqrt(v + EPS)


def _gelu(x):
    c = math.sqrt(2.0 / math.pi)
    t = jnp.tanh(x * (c + (c * 0.044715) * (x * x)))
    h = 0.5 * x
    return h + h * t


def _silu(y):
    h = 0.5 * y
    return h + h * jnp.tanh(h)


def _dot(a, b):
    return jnp.dot(a, b, preferred_element_type=F32)


def _own_block(i, body):
    return jax.lax.fori_loop(0, jnp.minimum(i + 1, 1), lambda _, c: body(i, c), 0)


def _kernel(x_hbm, mem0_hbm, wq_hbm, wk_hbm, wv_hbm, wo_hbm, w1_hbm, w2_hbm,
            w3_hbm, w4_hbm, out_hbm,
            xbuf, obuf, sbuf, mbuf, lhs, x1buf, hbuf, zc, w1, w2, w3t, w4t, wot, raw, wqkv, tmp,
            sems, sem_out):
    def x_copy(c):
        lo, rows = XCUTS[c], XCUTS[c + 1] - XCUTS[c]
        return pltpu.make_async_copy(x_hbm.at[pl.ds(lo, rows)], xbuf.at[pl.ds(lo, rows)],
                                     sems.at[SEM_X + c])

    def slab_copies(src, dst, sem_of):
        return [pltpu.make_async_copy(src.at[:, pl.ds(j * 128, 128)], dst.at[j], sems.at[sem_of(j)])
                for j in range(dst.shape[0])]

    w1_copies = slab_copies(w1_hbm, w1, lambda j: SEM_W1 + j)
    mem_copy = pltpu.make_async_copy(mem0_hbm, mbuf, sems.at[SEM_MEM])
    w2_copy = pltpu.make_async_copy(w2_hbm, w2, sems.at[SEM_W2])
    w3_copies = slab_copies(w3_hbm, w3t, lambda j: SEM_W3)
    w4_copies = slab_copies(w4_hbm, w4t, lambda j: SEM_W4)
    wo_copies = slab_copies(wo_hbm, wot, lambda j: SEM_WO)
    raw_copies = []
    for i in range(NP3):
        lo, hi = i * RC, (i + 1) * RC
        for w, src in enumerate((wq_hbm, wk_hbm, wv_hbm)):
            a, b = max(lo, w * D), min(hi, (w + 1) * D)
            if a < b:
                raw_copies.append(pltpu.make_async_copy(
                    src.at[pl.ds(a - w * D, b - a)], raw.at[pl.ds(a, b - a)], sems.at[SEM_RAW + i]))

    for cp in ([x_copy(0), x_copy(1)] + w1_copies + [x_copy(c) for c in range(2, len(XCUTS) - 1)]
               + [mem_copy, w2_copy] + w3_copies + w4_copies + raw_copies + wo_copies):
        cp.start(priority=1)

    sbuf[...] = jnp.zeros((SS, D), F32)
    hbuf[:, 0:HPAD, :] = jnp.zeros((NT, HPAD, 128), F32)
    hbuf[:, HPAD + S:HPAD + S + HPAD, :] = jnp.zeros((NT, HPAD, 128), F32)

    PPI = TM // SS

    def ln_piece(p):
        if isinstance(p, int):
            r0, l0 = p * SS, p * LROWS
        else:
            r0, l0 = pl.multiple_of(p * SS, SS), pl.multiple_of(p * LROWS, 16)
        xn = _ln(xbuf[pl.ds(r0, SS), :].astype(F32))
        lhs[pl.ds(l0 + M, XA), :] = xn[:XA].astype(BF16)
        lhs[pl.ds(l0 + 2 * M + XA, SS - XA), :] = xn[XA:].astype(BF16)
        return _ln(xn).astype(BF16)

    x_copy(0).wait()
    z0 = [ln_piece(0), ln_piece(1)]
    x_copy(1).wait()
    z0 = jnp.concatenate(z0 + [ln_piece(2), ln_piece(3)], axis=0)
    for n0 in range(0, NT, 2):
        w1_copies[n0].wait()
        w1_copies[n0 + 1].wait()
        for n in (n0, n0 + 1):
            hbuf[n, HPAD:HPAD + TM, :] = _gelu(_dot(z0, w1[n]))
    zc[...] = ln_piece(PPI)
    x_copy(2).wait()

    def p1(c, carry):
        z = zc[...]
        for q in range(P1N):
            p = PPI + c * P1N + q
            pn = jnp.minimum(p + 1, NSS - 1)
            r0 = pl.multiple_of(p * SS, SS)
            znext = ln_piece(pn)
            for n in range(NT):
                hbuf[n, pl.ds(r0 + HPAD, SS), :] = _gelu(_dot(z, w1[n]))
            z = znext
        zc[...] = z

        @pl.when(c == 0)
        def _():
            x_copy(3).wait()

        @pl.when(c == 1)
        def _():
            x_copy(4).wait()

        return carry

    jax.lax.fori_loop(0, (NSS - PPI) // P1N, p1, 0)

    w2_copy.wait()
    mem_copy.wait()
    lhs[0:M, :] = mbuf[...]
    P2U = 2

    def mix_rows(r0, pieces):
        rows = pieces * SS
        g = jnp.concatenate(
            [hbuf[n, pl.ds(r0 + (HPAD + sh), rows), :].astype(BF16)
             for n, sh in enumerate((-1, -1, 1, 1, -2, -2, 2, 2))], axis=1)
        l0 = pl.multiple_of((r0 // SS) * LROWS, 16)
        xn = jnp.concatenate(
            [lhs[pl.ds(l0 + q * LROWS + off, n), :].astype(F32)
             for q in range(pieces) for off, n in ((M, XA), (2 * M + XA, SS - XA))], axis=0)
        x1buf[pl.ds(r0, rows), :] = (xn + _dot(g, w2[...])).astype(BF16)

    def p2(cc, carry):
        for k in range(P2U):
            mix_rows(pl.multiple_of((cc * P2U + k) * TM, TM), PPI)
        return carry

    P2ROWS = S - NP3 * P3M
    jax.lax.fori_loop(0, P2ROWS // TM // P2U, p2, 0)

    def relayout_block(b, slot):
        w = b // (D // 16)
        r0 = pl.multiple_of((b % (D // 16)) * 8, 8)
        d0 = pl.multiple_of(b * 16, 16)
        blk = pltpu.bitcast(raw[pl.ds(d0, 16)], U32)
        for d in range(16):
            for j in range(2):
                tmp[slot, pl.ds(8 * j * PITCH + d, 8, stride=PITCH), :] = blk[d, 8 * j:8 * j + 8, :]
        for hp in range(16):
            a = tmp[slot, pl.ds(hp * PITCH, 8, stride=2), :]
            bb = tmp[slot, pl.ds(hp * PITCH + 1, 8, stride=2), :]
            wqkv[w * H + 2 * hp, pl.ds(r0, 8), :] = (a & U32(0xFFFF)) | (bb << 16)
            wqkv[w * H + 2 * hp + 1, pl.ds(r0, 8), :] = (a >> 16) | (bb & U32(0xFFFF0000))

    for cp in w3_copies + w4_copies:
        cp.wait()

    def p3(i, carry):
        nb = RC // 16
        r0 = pl.multiple_of(i * P3R, P3R)
        z = _ln(x1buf[pl.ds(r0, P3R), :].astype(F32)).astype(BF16)
        mix_rows(pl.multiple_of(P2ROWS + i * P3M, P3M), P3M // SS)
        done = 0
        us = []
        for k in range(NF + NT):
            if k < NF:
                us.append(_gelu(_dot(z, w3t[k])).astype(BF16))
                upto = 36 * (k + 1) // NF
            else:
                n = k - NF
                if n == 0:
                    u = jnp.concatenate(us, axis=1)
                y = x1buf[pl.ds(r0, P3R), n * 128:(n + 1) * 128].astype(F32) + _dot(u, w4t[n])
                x1buf[pl.ds(r0, P3R), n * 128:(n + 1) * 128] = _silu(y).astype(BF16)
                upto = min(nb, 36 + (nb - 36) * (n + 1) // 6)
            for b in range(done, upto):
                relayout_block(i * nb + b, b % NTMP)
            done = upto
        return carry

    def p3_outer(i, carry):
        c0 = pl.multiple_of(i * RC, 16)
        pltpu.make_async_copy(raw.at[pl.ds(c0, RC)], raw.at[pl.ds(c0, RC)], sems.at[SEM_RAW + i]).wait()
        return _own_block(i, p3)

    jax.lax.fori_loop(0, NP3, p3_outer, 0)

    for cp in wo_copies:
        cp.wait()

    ri = jax.lax.broadcasted_iota(jnp.int32, (2 * L, 128), 0)
    ci = jax.lax.broadcasted_iota(jnp.int32, (2 * L, 128), 1)
    second = ri >= L
    rr = jnp.where(second, ri - L, ri)
    cc = jnp.where(second, ci - L, ci)
    valid = (cc >= 0) & (cc < L) & ((rr < M) | (rr >= cc))
    cexp = (E ** -0.5) * math.log2(math.e)
    zpad = jnp.zeros((128 - 2 * L, E), F32)

    def wtile(idx):
        return pltpu.bitcast(wqkv[idx, 0:D // 2, :], BF16)

    GH = 8
    NG = H // GH

    def scores(q2, k2):
        kp = jnp.concatenate([k2, zpad], axis=0).astype(BF16)
        return jax.lax.dot_general(q2.astype(BF16), kp, (((1,), (1,)), ((), ())),
                                   preferred_element_type=F32)

    def softmax(s):
        s = jnp.where(valid, s, NEG)
        m = jnp.max(s, axis=1, keepdims=True)
        p = jnp.exp2((s - m) * cexp)
        l = jnp.sum(p, axis=1, keepdims=True)
        r = pl.reciprocal(l, approx=True)
        return p.astype(BF16), r * (2.0 - l * r)

    def half_step(h_in, carry_qkv, carry_o, fillers):
        step_a = carry_qkv is None
        new_qkv, new_o = {}, {}
        rows = {}

        def proj(t, h):
            y = _dot(h_in, wtile(t * H + h))
            if step_a:
                new_qkv[t, h] = y[L:]
                rows[t, h] = [y[:L]]
            else:
                rows[t, h] = [y[:M], carry_qkv[t, h], y[M:]]

        def pair(t, p):
            return jnp.concatenate(rows[t, 2 * p] + rows[t, 2 * p + 1], axis=0)

        def qk(g, half):
            for h in range(g * GH + half * GH // 2, g * GH + (half + 1) * GH // 2):
                proj(0, h)
                proj(1, h)

        def vproj(g):
            for h in range(g * GH, (g + 1) * GH):
                proj(2, h)

        def pairs(g):
            return range(g * GH // 2, (g + 1) * GH // 2)

        def s_stage(g):
            raw_s = [scores(pair(0, p), pair(1, p)) for p in pairs(g)]
            return [softmax(s) for s in raw_s]

        def pv_stage(g, pl_):
            og = []
            o2s = [_dot(pb, jnp.concatenate([pair(2, p), zpad], axis=0).astype(BF16))
                   for p, (pb, _) in zip(pairs(g), pl_)]
            for p, o2, (_, rl) in zip(pairs(g), o2s, pl_):
                o2 = o2 * rl
                for hh in range(2):
                    o = o2[hh * L:(hh + 1) * L]
                    if step_a:
                        new_o[2 * p + hh] = o[L - M:]
                        og.append(o[:L - M].astype(BF16))
                    else:
                        og.append(jnp.concatenate([o, carry_o[2 * p + hh]], axis=0).astype(BF16))
            return jnp.concatenate(og, axis=1)

        def wo_stage(g, ob, acc):
            part = jnp.concatenate(
                [_dot(ob, wot[n, g * GH * E:(g + 1) * GH * E, :]) for n in range(NT)], axis=1)
            return part if acc is None else acc + part

        acc = None
        qk(0, 0)
        qk(0, 1)
        for g in range(NG):
            last = g == NG - 1
            vproj(g)
            pl_ = s_stage(g)
            fillers[0]() if last else qk(g + 1, 0)
            ob = pv_stage(g, pl_)
            fillers[1]() if last else qk(g + 1, 1)
            acc = wo_stage(g, ob, acc)
        return acc, new_qkv, new_o

    def out_copy(jb):
        return pltpu.make_async_copy(obuf.at[pl.ds(pl.multiple_of(jb * SS, SS), SS)],
                                     out_hbm.at[pl.ds(pl.multiple_of((jb - 1) * SS, SS), SS)],
                                     sem_out)

    def combine(jb):
        t0 = pl.multiple_of(jnp.maximum(jb - 1, 0) * SS, SS)
        g = x1buf[pl.ds(t0, SS), :].astype(F32)
        x = xbuf[pl.ds(t0, SS), :].astype(F32)
        obuf[pl.ds(pl.multiple_of(jb * SS, SS), SS), :] = (x + sbuf[...] * g).astype(BF16)

    FS = (9, 18, 4)

    def superstep(j, carry):
        l0 = pl.multiple_of(j * LROWS, 16)
        f0 = pl.multiple_of(T0 + j * MF, 16)
        combine(j)

        x1 = x1buf[pl.ds(f0, MF), :].astype(F32)
        z = _ln(x1).astype(BF16)
        us = []

        def up(a, b):
            def f():
                for jj in range(a, b):
                    us.append(_gelu(_dot(z, w3t[jj])).astype(BF16))
            return f

        def down(a, b):
            def f():
                u = jnp.concatenate(us, axis=1)
                for n in range(a, b):
                    y = x1[:, n * 128:(n + 1) * 128] + _dot(u, w4t[n])
                    x1buf[pl.ds(f0, MF), n * 128:(n + 1) * 128] = _silu(y).astype(BF16)
            return f

        acc_a, cq, co = half_step(lhs[pl.ds(l0, M + XA), :], None, None,
                                  [up(0, FS[0]), up(FS[0], FS[1])])
        lhs[pl.ds(l0 + M + XA, M), :] = acc_a[:M].astype(BF16)
        sbuf[0:SEG - M, :] = acc_a[M:]
        up(FS[1], NF)()
        acc_b, _, _ = half_step(lhs[pl.ds(l0 + M + XA, M + SS - XA), :], cq, co,
                                [down(0, FS[2]), down(FS[2], NT)])
        lhs[pl.ds(l0 + LROWS, M), :] = acc_b[:M].astype(BF16)
        sbuf[SEG - M:SEG, :] = acc_b[L:]
        sbuf[SEG:SS, :] = acc_b[M:L]

        @pl.when(j > 0)
        def _():
            out_copy(j).start(priority=1)

        return carry

    jax.lax.fori_loop(0, NSS, superstep, 0)
    combine(NSS)
    out_copy(NSS).start(priority=1)
    pltpu.make_async_copy(out_hbm, out_hbm, sem_out).wait()


@jax.jit
def pallas_recurrent_scan__memory_aug_recurrent_mem_tr__mixer_s_mlp__prompt_kernel(
    A_x, A_mem0, A_Wq, A_Wk, A_Wv, A_Wo, A_seg_len, B_x, B_w1, B_w2, B_w3, B_w4,
):
    del A_seg_len, B_x
    assert A_x.shape == (1, S, D) and A_Wq.shape == (D, H, E)
    hbm = pl.BlockSpec(memory_space=pl.ANY)
    out = pl.pallas_call(
        _kernel,
        out_shape=jax.ShapeDtypeStruct((S, D), BF16),
        in_specs=[hbm] * 10,
        out_specs=hbm,
        scratch_shapes=[
            pltpu.VMEM((S, D), BF16),
            pltpu.VMEM((S + SS, D), BF16),
            pltpu.VMEM((SS, D), F32),
            pltpu.VMEM((M, D), BF16),
            pltpu.VMEM((NSS * LROWS + 16, D), BF16),
            pltpu.VMEM((S, D), BF16),
            pltpu.VMEM((NT, S + 2 * HPAD, 128), F32),
            pltpu.VMEM((SS, D), BF16),
            pltpu.VMEM((NT, D, 128), BF16),
            pltpu.VMEM((D, D), BF16),
            pltpu.VMEM((NF, D, 128), BF16),
            pltpu.VMEM((NT, FF, 128), BF16),
            pltpu.VMEM((NT, H * E, 128), BF16),
            pltpu.VMEM((3 * D, H, E), BF16),
            pltpu.VMEM((3 * H, D // 2 + WPAD, E), U32),
            pltpu.VMEM((NTMP, 16 * PITCH, 128), U32),
            pltpu.SemaphoreType.DMA((NSEM,)),
            pltpu.SemaphoreType.DMA,
        ],
        compiler_params=pltpu.CompilerParams(vmem_limit_bytes=120 * 1024 * 1024),
    )(A_x.reshape(S, D), A_mem0.reshape(M, D), A_Wq, A_Wk, A_Wv,
      A_Wo.reshape(H * E, D), B_w1, B_w2, B_w3, B_w4)
    return out.reshape(1, S, D)
```

```python
import math

import jax
import jax.numpy as jnp
import jax.experimental.pallas as pl
import jax.experimental.pallas.tpu as pltpu

F32 = jnp.float32
BF16 = jnp.bfloat16
U32 = jnp.uint32

S, D = 2048, 1024
H, E = 32, 128
M = 8
SEG = 32
FF = 3584
L = M + SEG
SS = 2 * SEG
NSS = S // SS
LROWS = SS + 2 * M
XA = 40
TM = 256
T0 = 512
MF = (S - T0) // NSS
NP3 = 4
P3R = T0 // NP3
RC = 3 * D // NP3
P3M = 128
NT = D // 128
NF = FF // 128
EPS = 1e-5
NEG = -1e30
PITCH = 20
NTMP = 2
WPAD = 8
HPAD = 8
P1N = 7
XCUTS = (0, 128, 320, 320 + 64 * P1N, 320 + 128 * P1N, S)

SEM_X = 0
SEM_W1 = SEM_X + len(XCUTS) - 1
SEM_MEM = SEM_W1 + NT // 2
SEM_W2, SEM_W3, SEM_W4, SEM_WO = SEM_MEM + 1, SEM_MEM + 2, SEM_MEM + 3, SEM_MEM + 4
SEM_RAW = SEM_WO + 1
NSEM = SEM_RAW + NP3


def _ln(x):
    m = jnp.mean(x, axis=-1, keepdims=True)
    xc = x - m
    v = jnp.mean(xc * xc, axis=-1, keepdims=True)
    return xc * jax.lax.rsqrt(v + EPS)


def _gelu(x):
    c = math.sqrt(2.0 / math.pi)
    t = jnp.tanh(x * (c + (c * 0.044715) * (x * x)))
    h = 0.5 * x
    return h + h * t


def _silu(y):
    h = 0.5 * y
    return h + h * jnp.tanh(h)


def _dot(a, b):
    return jnp.dot(a, b, preferred_element_type=F32)


def _own_block(i, body):
    return jax.lax.fori_loop(0, jnp.minimum(i + 1, 1), lambda _, c: body(i, c), 0)


def _kernel(x_hbm, mem0_hbm, wq_hbm, wk_hbm, wv_hbm, wo_hbm, w1_hbm, w2_hbm,
            w3_hbm, w4_hbm, out_hbm,
            xbuf, obuf, sbuf, mbuf, lhs, x1buf, hbuf, zc, w1, w2, w3t, w4t, wot, raw, wqkv, tmp,
            sems, sem_out):
    def x_copy(c):
        lo, rows = XCUTS[c], XCUTS[c + 1] - XCUTS[c]
        return pltpu.make_async_copy(x_hbm.at[pl.ds(lo, rows)], xbuf.at[pl.ds(lo, rows)],
                                     sems.at[SEM_X + c])

    def slab_copies(src, dst, sem_of):
        return [pltpu.make_async_copy(src.at[:, pl.ds(j * 128, 128)], dst.at[j], sems.at[sem_of(j)])
                for j in range(dst.shape[0])]

    w1_copies = [pltpu.make_async_copy(w1_hbm.at[:, pl.ds(j * 256, 256)], w1.at[j], sems.at[SEM_W1 + j])
                 for j in range(NT // 2)]

    def w1_tile(n):
        return w1[n // 2, :, (n % 2) * 128:(n % 2 + 1) * 128]

    mem_copy = pltpu.make_async_copy(mem0_hbm, mbuf, sems.at[SEM_MEM])
    w2_copy = pltpu.make_async_copy(w2_hbm, w2, sems.at[SEM_W2])
    w3_copies = slab_copies(w3_hbm, w3t, lambda j: SEM_W3)
    w4_copies = slab_copies(w4_hbm, w4t, lambda j: SEM_W4)
    wo_copies = slab_copies(wo_hbm, wot, lambda j: SEM_WO)
    raw_copies = []
    for i in range(NP3):
        lo, hi = i * RC, (i + 1) * RC
        for w, src in enumerate((wq_hbm, wk_hbm, wv_hbm)):
            a, b = max(lo, w * D), min(hi, (w + 1) * D)
            if a < b:
                raw_copies.append(pltpu.make_async_copy(
                    src.at[pl.ds(a - w * D, b - a)], raw.at[pl.ds(a, b - a)], sems.at[SEM_RAW + i]))

    for cp in ([x_copy(0), x_copy(1)] + w1_copies + [x_copy(c) for c in range(2, len(XCUTS) - 1)]
               + [mem_copy, w2_copy] + w3_copies + w4_copies + raw_copies + wo_copies):
        cp.start(priority=1)

    sbuf[...] = jnp.zeros((SS, D), F32)
    hbuf[:, 0:HPAD, :] = jnp.zeros((NT, HPAD, 128), F32)
    hbuf[:, HPAD + S:HPAD + S + HPAD, :] = jnp.zeros((NT, HPAD, 128), F32)

    PPI = TM // SS

    def ln_piece(p):
        if isinstance(p, int):
            r0, l0 = p * SS, p * LROWS
        else:
            r0, l0 = pl.multiple_of(p * SS, SS), pl.multiple_of(p * LROWS, 16)
        xn = _ln(xbuf[pl.ds(r0, SS), :].astype(F32))
        lhs[pl.ds(l0 + M, XA), :] = xn[:XA].astype(BF16)
        lhs[pl.ds(l0 + 2 * M + XA, SS - XA), :] = xn[XA:].astype(BF16)
        return _ln(xn).astype(BF16)

    x_copy(0).wait()
    z0 = [ln_piece(0), ln_piece(1)]
    x_copy(1).wait()
    z0 = jnp.concatenate(z0 + [ln_piece(2), ln_piece(3)], axis=0)
    for n0 in range(0, NT, 2):
        w1_copies[n0 // 2].wait()
        for n in (n0, n0 + 1):
            hbuf[n, HPAD:HPAD + TM, :] = _gelu(_dot(z0, w1_tile(n)))
    zc[...] = ln_piece(PPI)
    x_copy(2).wait()

    def p1(c, carry):
        z = zc[...]
        for q in range(P1N):
            p = PPI + c * P1N + q
            pn = jnp.minimum(p + 1, NSS - 1)
            r0 = pl.multiple_of(p * SS, SS)
            znext = ln_piece(pn)
            for n in range(NT):
                hbuf[n, pl.ds(r0 + HPAD, SS), :] = _gelu(_dot(z, w1_tile(n)))
            z = znext
        zc[...] = z

        @pl.when(c == 0)
        def _():
            x_copy(3).wait()

        @pl.when(c == 1)
        def _():
            x_copy(4).wait()

        return carry

    jax.lax.fori_loop(0, (NSS - PPI) // P1N, p1, 0)

    w2_copy.wait()
    mem_copy.wait()
    lhs[0:M, :] = mbuf[...]
    P2U = 2

    def mix_rows(r0, pieces):
        rows = pieces * SS
        g = jnp.concatenate(
            [hbuf[n, pl.ds(r0 + (HPAD + sh), rows), :].astype(BF16)
             for n, sh in enumerate((-1, -1, 1, 1, -2, -2, 2, 2))], axis=1)
        l0 = pl.multiple_of((r0 // SS) * LROWS, 16)
        xn = jnp.concatenate(
            [lhs[pl.ds(l0 + q * LROWS + off, n), :].astype(F32)
             for q in range(pieces) for off, n in ((M, XA), (2 * M + XA, SS - XA))], axis=0)
        x1buf[pl.ds(r0, rows), :] = (xn + _dot(g, w2[...])).astype(BF16)

    def p2(cc, carry):
        for k in range(P2U):
            mix_rows(pl.multiple_of((cc * P2U + k) * TM, TM), PPI)
        return carry

    P2ROWS = S - NP3 * P3M
    jax.lax.fori_loop(0, P2ROWS // TM // P2U, p2, 0)

    def relayout_block(b, slot):
        w = b // (D // 16)
        r0 = pl.multiple_of((b % (D // 16)) * 8, 8)
        d0 = pl.multiple_of(b * 16, 16)
        blk = pltpu.bitcast(raw[pl.ds(d0, 16)], U32)
        for d in range(16):
            for j in range(2):
                tmp[slot, pl.ds(8 * j * PITCH + d, 8, stride=PITCH), :] = blk[d, 8 * j:8 * j + 8, :]
        for hp in range(16):
            a = tmp[slot, pl.ds(hp * PITCH, 8, stride=2), :]
            bb = tmp[slot, pl.ds(hp * PITCH + 1, 8, stride=2), :]
            wqkv[w * H + 2 * hp, pl.ds(r0, 8), :] = (a & U32(0xFFFF)) | (bb << 16)
            wqkv[w * H + 2 * hp + 1, pl.ds(r0, 8), :] = (a >> 16) | (bb & U32(0xFFFF0000))

    for cp in w3_copies + w4_copies:
        cp.wait()

    def p3(i, carry):
        nb = RC // 16
        r0 = pl.multiple_of(i * P3R, P3R)
        z = _ln(x1buf[pl.ds(r0, P3R), :].astype(F32)).astype(BF16)
        mix_rows(pl.multiple_of(P2ROWS + i * P3M, P3M), P3M // SS)
        done = 0
        us = []
        for k in range(NF + NT):
            if k < NF:
                us.append(_gelu(_dot(z, w3t[k])).astype(BF16))
                upto = 36 * (k + 1) // NF
            else:
                n = k - NF
                if n == 0:
                    u = jnp.concatenate(us, axis=1)
                y = x1buf[pl.ds(r0, P3R), n * 128:(n + 1) * 128].astype(F32) + _dot(u, w4t[n])
                x1buf[pl.ds(r0, P3R), n * 128:(n + 1) * 128] = _silu(y).astype(BF16)
                upto = min(nb, 36 + (nb - 36) * (n + 1) // 6)
            for b in range(done, upto):
                relayout_block(i * nb + b, b % NTMP)
            done = upto
        return carry

    def p3_outer(i, carry):
        c0 = pl.multiple_of(i * RC, 16)
        pltpu.make_async_copy(raw.at[pl.ds(c0, RC)], raw.at[pl.ds(c0, RC)], sems.at[SEM_RAW + i]).wait()
        return _own_block(i, p3)

    jax.lax.fori_loop(0, NP3, p3_outer, 0)

    for cp in wo_copies:
        cp.wait()

    ri = jax.lax.broadcasted_iota(jnp.int32, (2 * L, 128), 0)
    ci = jax.lax.broadcasted_iota(jnp.int32, (2 * L, 128), 1)
    second = ri >= L
    rr = jnp.where(second, ri - L, ri)
    cc = jnp.where(second, ci - L, ci)
    valid = (cc >= 0) & (cc < L) & ((rr < M) | (rr >= cc))
    cexp = (E ** -0.5) * math.log2(math.e)
    zpad = jnp.zeros((128 - 2 * L, E), F32)

    def wtile(idx):
        return pltpu.bitcast(wqkv[idx, 0:D // 2, :], BF16)

    GH = 8
    NG = H // GH

    def scores(q2, k2):
        kp = jnp.concatenate([k2, zpad], axis=0).astype(BF16)
        return jax.lax.dot_general(q2.astype(BF16), kp, (((1,), (1,)), ((), ())),
                                   preferred_element_type=F32)

    def softmax(s):
        s = jnp.where(valid, s, NEG)
        m = jnp.max(s, axis=1, keepdims=True)
        p = jnp.exp2((s - m) * cexp)
        l = jnp.sum(p, axis=1, keepdims=True)
        r = pl.reciprocal(l, approx=True)
        return p.astype(BF16), r * (2.0 - l * r)

    def half_step(h_in, carry_qkv, carry_o, fillers):
        step_a = carry_qkv is None
        new_qkv, new_o = {}, {}
        rows = {}

        def proj(t, h):
            y = _dot(h_in, wtile(t * H + h))
            if step_a:
                new_qkv[t, h] = y[L:]
                rows[t, h] = [y[:L]]
            else:
                rows[t, h] = [y[:M], carry_qkv[t, h], y[M:]]

        def pair(t, p):
            return jnp.concatenate(rows[t, 2 * p] + rows[t, 2 * p + 1], axis=0)

        def qk(g, half):
            for h in range(g * GH + half * GH // 2, g * GH + (half + 1) * GH // 2):
                proj(0, h)
                proj(1, h)

        def vproj(g):
            for h in range(g * GH, (g + 1) * GH):
                proj(2, h)

        def pairs(g):
            return range(g * GH // 2, (g + 1) * GH // 2)

        def s_stage(g):
            raw_s = [scores(pair(0, p), pair(1, p)) for p in pairs(g)]
            return [softmax(s) for s in raw_s]

        def pv_stage(g, pl_):
            og = []
            o2s = [_dot(pb, jnp.concatenate([pair(2, p), zpad], axis=0).astype(BF16))
                   for p, (pb, _) in zip(pairs(g), pl_)]
            for p, o2, (_, rl) in zip(pairs(g), o2s, pl_):
                o2 = o2 * rl
                for hh in range(2):
                    o = o2[hh * L:(hh + 1) * L]
                    if step_a:
                        new_o[2 * p + hh] = o[L - M:]
                        og.append(o[:L - M].astype(BF16))
                    else:
                        og.append(jnp.concatenate([o, carry_o[2 * p + hh]], axis=0).astype(BF16))
            return jnp.concatenate(og, axis=1)

        def wo_stage(g, ob, acc):
            part = jnp.concatenate(
                [_dot(ob, wot[n, g * GH * E:(g + 1) * GH * E, :]) for n in range(NT)], axis=1)
            return part if acc is None else acc + part

        acc = None
        qk(0, 0)
        qk(0, 1)
        for g in range(NG):
            last = g == NG - 1
            vproj(g)
            pl_ = s_stage(g)
            fillers[0]() if last else qk(g + 1, 0)
            ob = pv_stage(g, pl_)
            fillers[1]() if last else qk(g + 1, 1)
            acc = wo_stage(g, ob, acc)
        return acc, new_qkv, new_o

    def out_copy(jb):
        return pltpu.make_async_copy(obuf.at[pl.ds(pl.multiple_of(jb * SS, SS), SS)],
                                     out_hbm.at[pl.ds(pl.multiple_of((jb - 1) * SS, SS), SS)],
                                     sem_out)

    def combine(jb):
        t0 = pl.multiple_of(jnp.maximum(jb - 1, 0) * SS, SS)
        g = x1buf[pl.ds(t0, SS), :].astype(F32)
        x = xbuf[pl.ds(t0, SS), :].astype(F32)
        obuf[pl.ds(pl.multiple_of(jb * SS, SS), SS), :] = (x + sbuf[...] * g).astype(BF16)

    FS = (9, 18, 4)

    def superstep(j, carry):
        l0 = pl.multiple_of(j * LROWS, 16)
        f0 = pl.multiple_of(T0 + j * MF, 16)
        combine(j)

        x1 = x1buf[pl.ds(f0, MF), :].astype(F32)
        z = _ln(x1).astype(BF16)
        us = []

        def up(a, b):
            def f():
                for jj in range(a, b):
                    us.append(_gelu(_dot(z, w3t[jj])).astype(BF16))
            return f

        def down(a, b):
            def f():
                u = jnp.concatenate(us, axis=1)
                for n in range(a, b):
                    y = x1[:, n * 128:(n + 1) * 128] + _dot(u, w4t[n])
                    x1buf[pl.ds(f0, MF), n * 128:(n + 1) * 128] = _silu(y).astype(BF16)
            return f

        acc_a, cq, co = half_step(lhs[pl.ds(l0, M + XA), :], None, None,
                                  [up(0, FS[0]), up(FS[0], FS[1])])
        lhs[pl.ds(l0 + M + XA, M), :] = acc_a[:M].astype(BF16)
        sbuf[0:SEG - M, :] = acc_a[M:]
        up(FS[1], NF)()
        acc_b, _, _ = half_step(lhs[pl.ds(l0 + M + XA, M + SS - XA), :], cq, co,
                                [down(0, FS[2]), down(FS[2], NT)])
        lhs[pl.ds(l0 + LROWS, M), :] = acc_b[:M].astype(BF16)
        sbuf[SEG - M:SEG, :] = acc_b[L:]
        sbuf[SEG:SS, :] = acc_b[M:L]

        @pl.when(j > 0)
        def _():
            out_copy(j).start(priority=1)

        return carry

    jax.lax.fori_loop(0, NSS, superstep, 0)
    combine(NSS)
    out_copy(NSS).start(priority=1)
    pltpu.make_async_copy(out_hbm, out_hbm, sem_out).wait()


@jax.jit
def pallas_recurrent_scan__memory_aug_recurrent_mem_tr__mixer_s_mlp__prompt_kernel(
    A_x, A_mem0, A_Wq, A_Wk, A_Wv, A_Wo, A_seg_len, B_x, B_w1, B_w2, B_w3, B_w4,
):
    del A_seg_len, B_x
    assert A_x.shape == (1, S, D) and A_Wq.shape == (D, H, E)
    hbm = pl.BlockSpec(memory_space=pl.ANY)
    out = pl.pallas_call(
        _kernel,
        out_shape=jax.ShapeDtypeStruct((S, D), BF16),
        in_specs=[hbm] * 10,
        out_specs=hbm,
        scratch_shapes=[
            pltpu.VMEM((S, D), BF16),
            pltpu.VMEM((S + SS, D), BF16),
            pltpu.VMEM((SS, D), F32),
            pltpu.VMEM((M, D), BF16),
            pltpu.VMEM((NSS * LROWS + 16, D), BF16),
            pltpu.VMEM((S, D), BF16),
            pltpu.VMEM((NT, S + 2 * HPAD, 128), F32),
            pltpu.VMEM((SS, D), BF16),
            pltpu.VMEM((NT // 2, D, 256), BF16),
            pltpu.VMEM((D, D), BF16),
            pltpu.VMEM((NF, D, 128), BF16),
            pltpu.VMEM((NT, FF, 128), BF16),
            pltpu.VMEM((NT, H * E, 128), BF16),
            pltpu.VMEM((3 * D, H, E), BF16),
            pltpu.VMEM((3 * H, D // 2 + WPAD, E), U32),
            pltpu.VMEM((NTMP, 16 * PITCH, 128), U32),
            pltpu.SemaphoreType.DMA((NSEM,)),
            pltpu.SemaphoreType.DMA,
        ],
        compiler_params=pltpu.CompilerParams(vmem_limit_bytes=120 * 1024 * 1024),
    )(A_x.reshape(S, D), A_mem0.reshape(M, D), A_Wq, A_Wk, A_Wv,
      A_Wo.reshape(H * E, D), B_w1, B_w2, B_w3, B_w4)
    return out.reshape(1, S, D)
```

```python
import math

import jax
import jax.numpy as jnp
import jax.experimental.pallas as pl
import jax.experimental.pallas.tpu as pltpu

F32 = jnp.float32
BF16 = jnp.bfloat16
U32 = jnp.uint32

S, D = 2048, 1024
H, E = 32, 128
M = 8
SEG = 32
FF = 3584
L = M + SEG
SS = 2 * SEG
NSS = S // SS
LROWS = SS + 2 * M
XA = 40
TM = 256
T0 = 512
MF = (S - T0) // NSS
NP3 = 4
P3R = T0 // NP3
RC = 3 * D // NP3
P3M = 128
NT = D // 128
NF = FF // 128
EPS = 1e-5
NEG = -1e30
PITCH = 20
NTMP = 2
WPAD = 8
HPAD = 8
P1N = 7
XCUTS = (0, 128, 320, 320 + 64 * P1N, 320 + 128 * P1N, S)

SEM_X = 0
SEM_W1 = SEM_X + len(XCUTS) - 1
SEM_MEM = SEM_W1 + NT // 2
SEM_W2, SEM_W3, SEM_W4, SEM_WO = SEM_MEM + 1, SEM_MEM + 2, SEM_MEM + 3, SEM_MEM + 4
SEM_RAW = SEM_WO + 1
NSEM = SEM_RAW + NP3


def _ln(x):
    m = jnp.mean(x, axis=-1, keepdims=True)
    xc = x - m
    v = jnp.mean(xc * xc, axis=-1, keepdims=True)
    return xc * jax.lax.rsqrt(v + EPS)


def _gelu(x):
    c = math.sqrt(2.0 / math.pi)
    t = jnp.tanh(x * (c + (c * 0.044715) * (x * x)))
    h = 0.5 * x
    return h + h * t


def _silu(y):
    h = 0.5 * y
    return h + h * jnp.tanh(h)


def _dot(a, b):
    return jnp.dot(a, b, preferred_element_type=F32)


def _own_block(i, body):
    return jax.lax.fori_loop(0, jnp.minimum(i + 1, 1), lambda _, c: body(i, c), 0)


def _kernel(x_hbm, mem0_hbm, wq_hbm, wk_hbm, wv_hbm, wo_hbm, w1_hbm, w2_hbm,
            w3_hbm, w4_hbm, out_hbm,
            xbuf, obuf, sbuf, mbuf, lhs, x1buf, hbuf, zc, w1, w2, w3t, w4t, wot, raw, wqkv, tmp,
            sems, sem_out):
    def x_copy(c):
        lo, rows = XCUTS[c], XCUTS[c + 1] - XCUTS[c]
        return pltpu.make_async_copy(x_hbm.at[pl.ds(lo, rows)], xbuf.at[pl.ds(lo, rows)],
                                     sems.at[SEM_X + c])

    def slab_copies(src, dst, sem_of):
        return [pltpu.make_async_copy(src.at[:, pl.ds(j * 128, 128)], dst.at[j], sems.at[sem_of(j)])
                for j in range(dst.shape[0])]

    w1_copies = [pltpu.make_async_copy(w1_hbm.at[:, pl.ds(j * 256, 256)], w1.at[j], sems.at[SEM_W1 + j])
                 for j in range(NT // 2)]

    def w1_tile(n):
        return w1[n // 2, :, (n % 2) * 128:(n % 2 + 1) * 128]

    mem_copy = pltpu.make_async_copy(mem0_hbm, mbuf, sems.at[SEM_MEM])
    w2_copies = [pltpu.make_async_copy(w2_hbm.at[:, pl.ds(j * 256, 256)], w2.at[j], sems.at[SEM_W2])
                 for j in range(NT // 2)]
    w3_copies = slab_copies(w3_hbm, w3t, lambda j: SEM_W3)
    w4_copies = slab_copies(w4_hbm, w4t, lambda j: SEM_W4)
    wo_copies = slab_copies(wo_hbm, wot, lambda j: SEM_WO)
    raw_copies = []
    for i in range(NP3):
        lo, hi = i * RC, (i + 1) * RC
        for w, src in enumerate((wq_hbm, wk_hbm, wv_hbm)):
            a, b = max(lo, w * D), min(hi, (w + 1) * D)
            if a < b:
                raw_copies.append(pltpu.make_async_copy(
                    src.at[pl.ds(a - w * D, b - a)], raw.at[pl.ds(a, b - a)], sems.at[SEM_RAW + i]))

    for cp in ([x_copy(0), x_copy(1)] + w1_copies + [x_copy(c) for c in range(2, len(XCUTS) - 1)]
               + [mem_copy] + w2_copies + w3_copies + w4_copies + raw_copies + wo_copies):
        cp.start(priority=1)

    sbuf[...] = jnp.zeros((SS, D), F32)
    hbuf[:, 0:HPAD, :] = jnp.zeros((NT, HPAD, 128), F32)
    hbuf[:, HPAD + S:HPAD + S + HPAD, :] = jnp.zeros((NT, HPAD, 128), F32)

    PPI = TM // SS

    def ln_piece(p):
        if isinstance(p, int):
            r0, l0 = p * SS, p * LROWS
        else:
            r0, l0 = pl.multiple_of(p * SS, SS), pl.multiple_of(p * LROWS, 16)
        xn = _ln(xbuf[pl.ds(r0, SS), :].astype(F32))
        lhs[pl.ds(l0 + M, XA), :] = xn[:XA].astype(BF16)
        lhs[pl.ds(l0 + 2 * M + XA, SS - XA), :] = xn[XA:].astype(BF16)
        return _ln(xn).astype(BF16)

    x_copy(0).wait()
    z0 = [ln_piece(0), ln_piece(1)]
    x_copy(1).wait()
    z0 = jnp.concatenate(z0 + [ln_piece(2), ln_piece(3)], axis=0)
    for n0 in range(0, NT, 2):
        w1_copies[n0 // 2].wait()
        for n in (n0, n0 + 1):
            hbuf[n, HPAD:HPAD + TM, :] = _gelu(_dot(z0, w1_tile(n)))
    zc[...] = ln_piece(PPI)
    x_copy(2).wait()

    def p1(c, carry):
        z = zc[...]
        for q in range(P1N):
            p = PPI + c * P1N + q
            pn = jnp.minimum(p + 1, NSS - 1)
            r0 = pl.multiple_of(p * SS, SS)
            znext = ln_piece(pn)
            for n in range(NT):
                hbuf[n, pl.ds(r0 + HPAD, SS), :] = _gelu(_dot(z, w1_tile(n)))
            z = znext
        zc[...] = z

        @pl.when(c == 0)
        def _():
            x_copy(3).wait()

        @pl.when(c == 1)
        def _():
            x_copy(4).wait()

        return carry

    jax.lax.fori_loop(0, (NSS - PPI) // P1N, p1, 0)

    for cp in w2_copies:
        cp.wait()
    mem_copy.wait()
    lhs[0:M, :] = mbuf[...]
    P2U = 2

    def mix_rows(r0, pieces):
        rows = pieces * SS
        g = jnp.concatenate(
            [hbuf[n, pl.ds(r0 + (HPAD + sh), rows), :].astype(BF16)
             for n, sh in enumerate((-1, -1, 1, 1, -2, -2, 2, 2))], axis=1)
        l0 = pl.multiple_of((r0 // SS) * LROWS, 16)
        xn = jnp.concatenate(
            [lhs[pl.ds(l0 + q * LROWS + off, n), :].astype(F32)
             for q in range(pieces) for off, n in ((M, XA), (2 * M + XA, SS - XA))], axis=0)
        hs = jnp.concatenate([_dot(g, w2[j]) for j in range(NT // 2)], axis=1)
        x1buf[pl.ds(r0, rows), :] = (xn + hs).astype(BF16)

    def p2(cc, carry):
        for k in range(P2U):
            mix_rows(pl.multiple_of((cc * P2U + k) * TM, TM), PPI)
        return carry

    P2ROWS = S - NP3 * P3M
    jax.lax.fori_loop(0, P2ROWS // TM // P2U, p2, 0)

    def relayout_block(b, slot):
        w = b // (D // 16)
        r0 = pl.multiple_of((b % (D // 16)) * 8, 8)
        d0 = pl.multiple_of(b * 16, 16)
        blk = pltpu.bitcast(raw[pl.ds(d0, 16)], U32)
        for d in range(16):
            for j in range(2):
                tmp[slot, pl.ds(8 * j * PITCH + d, 8, stride=PITCH), :] = blk[d, 8 * j:8 * j + 8, :]
        for hp in range(16):
            a = tmp[slot, pl.ds(hp * PITCH, 8, stride=2), :]
            bb = tmp[slot, pl.ds(hp * PITCH + 1, 8, stride=2), :]
            wqkv[w * H + 2 * hp, pl.ds(r0, 8), :] = (a & U32(0xFFFF)) | (bb << 16)
            wqkv[w * H + 2 * hp + 1, pl.ds(r0, 8), :] = (a >> 16) | (bb & U32(0xFFFF0000))

    for cp in w3_copies + w4_copies:
        cp.wait()

    def p3(i, carry):
        nb = RC // 16
        r0 = pl.multiple_of(i * P3R, P3R)
        z = _ln(x1buf[pl.ds(r0, P3R), :].astype(F32)).astype(BF16)
        mix_rows(pl.multiple_of(P2ROWS + i * P3M, P3M), P3M // SS)
        done = 0
        us = []
        for k in range(NF + NT):
            if k < NF:
                us.append(_gelu(_dot(z, w3t[k])).astype(BF16))
                upto = 36 * (k + 1) // NF
            else:
                n = k - NF
                if n == 0:
                    u = jnp.concatenate(us, axis=1)
                y = x1buf[pl.ds(r0, P3R), n * 128:(n + 1) * 128].astype(F32) + _dot(u, w4t[n])
                x1buf[pl.ds(r0, P3R), n * 128:(n + 1) * 128] = _silu(y).astype(BF16)
                upto = min(nb, 36 + (nb - 36) * (n + 1) // 6)
            for b in range(done, upto):
                relayout_block(i * nb + b, b % NTMP)
            done = upto
        return carry

    def p3_outer(i, carry):
        c0 = pl.multiple_of(i * RC, 16)
        pltpu.make_async_copy(raw.at[pl.ds(c0, RC)], raw.at[pl.ds(c0, RC)], sems.at[SEM_RAW + i]).wait()
        return _own_block(i, p3)

    jax.lax.fori_loop(0, NP3, p3_outer, 0)

    for cp in wo_copies:
        cp.wait()

    ri = jax.lax.broadcasted_iota(jnp.int32, (2 * L, 128), 0)
    ci = jax.lax.broadcasted_iota(jnp.int32, (2 * L, 128), 1)
    second = ri >= L
    rr = jnp.where(second, ri - L, ri)
    cc = jnp.where(second, ci - L, ci)
    valid = (cc >= 0) & (cc < L) & ((rr < M) | (rr >= cc))
    cexp = (E ** -0.5) * math.log2(math.e)
    zpad = jnp.zeros((128 - 2 * L, E), F32)

    def wtile(idx):
        return pltpu.bitcast(wqkv[idx, 0:D // 2, :], BF16)

    GH = 8
    NG = H // GH

    def scores(q2, k2):
        kp = jnp.concatenate([k2, zpad], axis=0).astype(BF16)
        return jax.lax.dot_general(q2.astype(BF16), kp, (((1,), (1,)), ((), ())),
                                   preferred_element_type=F32)

    def softmax(s):
        s = jnp.where(valid, s, NEG)
        m = jnp.max(s, axis=1, keepdims=True)
        p = jnp.exp2((s - m) * cexp)
        l = jnp.sum(p, axis=1, keepdims=True)
        r = pl.reciprocal(l, approx=True)
        return p.astype(BF16), r * (2.0 - l * r)

    def half_step(h_in, carry_qkv, carry_o, fillers):
        step_a = carry_qkv is None
        new_qkv, new_o = {}, {}
        rows = {}

        def proj(t, h):
            y = _dot(h_in, wtile(t * H + h))
            if step_a:
                new_qkv[t, h] = y[L:]
                rows[t, h] = [y[:L]]
            else:
                rows[t, h] = [y[:M], carry_qkv[t, h], y[M:]]

        def pair(t, p):
            return jnp.concatenate(rows[t, 2 * p] + rows[t, 2 * p + 1], axis=0)

        def qk(g, half):
            for h in range(g * GH + half * GH // 2, g * GH + (half + 1) * GH // 2):
                proj(0, h)
                proj(1, h)

        def vproj(g):
            for h in range(g * GH, (g + 1) * GH):
                proj(2, h)

        def pairs(g):
            return range(g * GH // 2, (g + 1) * GH // 2)

        def s_stage(g):
            raw_s = [scores(pair(0, p), pair(1, p)) for p in pairs(g)]
            return [softmax(s) for s in raw_s]

        def pv_stage(g, pl_):
            og = []
            o2s = [_dot(pb, jnp.concatenate([pair(2, p), zpad], axis=0).astype(BF16))
                   for p, (pb, _) in zip(pairs(g), pl_)]
            for p, o2, (_, rl) in zip(pairs(g), o2s, pl_):
                o2 = o2 * rl
                for hh in range(2):
                    o = o2[hh * L:(hh + 1) * L]
                    if step_a:
                        new_o[2 * p + hh] = o[L - M:]
                        og.append(o[:L - M].astype(BF16))
                    else:
                        og.append(jnp.concatenate([o, carry_o[2 * p + hh]], axis=0).astype(BF16))
            return jnp.concatenate(og, axis=1)

        def wo_stage(g, ob, acc):
            part = jnp.concatenate(
                [_dot(ob, wot[n, g * GH * E:(g + 1) * GH * E, :]) for n in range(NT)], axis=1)
            return part if acc is None else acc + part

        acc = None
        qk(0, 0)
        qk(0, 1)
        for g in range(NG):
            last = g == NG - 1
            vproj(g)
            pl_ = s_stage(g)
            fillers[0]() if last else qk(g + 1, 0)
            ob = pv_stage(g, pl_)
            fillers[1]() if last else qk(g + 1, 1)
            acc = wo_stage(g, ob, acc)
        return acc, new_qkv, new_o

    def out_copy(jb):
        return pltpu.make_async_copy(obuf.at[pl.ds(pl.multiple_of(jb * SS, SS), SS)],
                                     out_hbm.at[pl.ds(pl.multiple_of((jb - 1) * SS, SS), SS)],
                                     sem_out)

    def combine(jb):
        t0 = pl.multiple_of(jnp.maximum(jb - 1, 0) * SS, SS)
        g = x1buf[pl.ds(t0, SS), :].astype(F32)
        x = xbuf[pl.ds(t0, SS), :].astype(F32)
        obuf[pl.ds(pl.multiple_of(jb * SS, SS), SS), :] = (x + sbuf[...] * g).astype(BF16)

    FS = (9, 18, 4)

    def superstep(j, carry):
        l0 = pl.multiple_of(j * LROWS, 16)
        f0 = pl.multiple_of(T0 + j * MF, 16)
        combine(j)

        x1 = x1buf[pl.ds(f0, MF), :].astype(F32)
        z = _ln(x1).astype(BF16)
        us = []

        def up(a, b):
            def f():
                for jj in range(a, b):
                    us.append(_gelu(_dot(z, w3t[jj])).astype(BF16))
            return f

        def down(a, b):
            def f():
                u = jnp.concatenate(us, axis=1)
                for n in range(a, b):
                    y = x1[:, n * 128:(n + 1) * 128] + _dot(u, w4t[n])
                    x1buf[pl.ds(f0, MF), n * 128:(n + 1) * 128] = _silu(y).astype(BF16)
            return f

        acc_a, cq, co = half_step(lhs[pl.ds(l0, M + XA), :], None, None,
                                  [up(0, FS[0]), up(FS[0], FS[1])])
        lhs[pl.ds(l0 + M + XA, M), :] = acc_a[:M].astype(BF16)
        sbuf[0:SEG - M, :] = acc_a[M:]
        up(FS[1], NF)()
        acc_b, _, _ = half_step(lhs[pl.ds(l0 + M + XA, M + SS - XA), :], cq, co,
                                [down(0, FS[2]), down(FS[2], NT)])
        lhs[pl.ds(l0 + LROWS, M), :] = acc_b[:M].astype(BF16)
        sbuf[SEG - M:SEG, :] = acc_b[L:]
        sbuf[SEG:SS, :] = acc_b[M:L]

        @pl.when(j > 0)
        def _():
            out_copy(j).start(priority=1)

        return carry

    jax.lax.fori_loop(0, NSS, superstep, 0)
    combine(NSS)
    out_copy(NSS).start(priority=1)
    pltpu.make_async_copy(out_hbm, out_hbm, sem_out).wait()


@jax.jit
def pallas_recurrent_scan__memory_aug_recurrent_mem_tr__mixer_s_mlp__prompt_kernel(
    A_x, A_mem0, A_Wq, A_Wk, A_Wv, A_Wo, A_seg_len, B_x, B_w1, B_w2, B_w3, B_w4,
):
    del A_seg_len, B_x
    assert A_x.shape == (1, S, D) and A_Wq.shape == (D, H, E)
    hbm = pl.BlockSpec(memory_space=pl.ANY)
    out = pl.pallas_call(
        _kernel,
        out_shape=jax.ShapeDtypeStruct((S, D), BF16),
        in_specs=[hbm] * 10,
        out_specs=hbm,
        scratch_shapes=[
            pltpu.VMEM((S, D), BF16),
            pltpu.VMEM((S + SS, D), BF16),
            pltpu.VMEM((SS, D), F32),
            pltpu.VMEM((M, D), BF16),
            pltpu.VMEM((NSS * LROWS + 16, D), BF16),
            pltpu.VMEM((S, D), BF16),
            pltpu.VMEM((NT, S + 2 * HPAD, 128), F32),
            pltpu.VMEM((SS, D), BF16),
            pltpu.VMEM((NT // 2, D, 256), BF16),
            pltpu.VMEM((NT // 2, D, 256), BF16),
            pltpu.VMEM((NF, D, 128), BF16),
            pltpu.VMEM((NT, FF, 128), BF16),
            pltpu.VMEM((NT, H * E, 128), BF16),
            pltpu.VMEM((3 * D, H, E), BF16),
            pltpu.VMEM((3 * H, D // 2 + WPAD, E), U32),
            pltpu.VMEM((NTMP, 16 * PITCH, 128), U32),
            pltpu.SemaphoreType.DMA((NSEM,)),
            pltpu.SemaphoreType.DMA,
        ],
        compiler_params=pltpu.CompilerParams(vmem_limit_bytes=120 * 1024 * 1024),
    )(A_x.reshape(S, D), A_mem0.reshape(M, D), A_Wq, A_Wk, A_Wv,
      A_Wo.reshape(H * E, D), B_w1, B_w2, B_w3, B_w4)
    return out.reshape(1, S, D)
```
